```python
import os as _os
_os.environ.setdefault('JAX_PLATFORMS', 'cpu')
import jax
import jax.numpy as jnp

def _softmax(x, axis=-1):
    return jax.nn.softmax(x, axis=axis)

def _gelu(x):
    return jax.nn.gelu(x, approximate=True)

def _silu(x):
    return jax.nn.silu(x)

def _sigmoid(x):
    return jax.nn.sigmoid(x)

def _layernorm(x, axis=-1, eps=1e-05):
    m = jnp.mean(x, axis=axis, keepdims=True)
    v = jnp.var(x, axis=axis, keepdims=True)
    return (x - m) / jnp.sqrt(v + eps)

def _scatter_add(tgt, idx, src, axis=0):
    return tgt.at[idx].add(src)

def _segment_sum(src, seg, n):
    return jax.ops.segment_sum(src, seg, n)

class _Rng:

    def __init__(self, key):
        self._k = key

    def _next(self):
        self._k, sub = jax.random.split(self._k)
        return sub

    def normal(self, shape):
        return jax.random.normal(self._next(), shape, dtype=jnp.bfloat16)

    def randint(self, lo, hi, shape):
        return jax.random.randint(self._next(), shape, lo, hi, dtype=jnp.int32)

    def uniform(self, shape, lo=0.0, hi=1.0):
        return jax.random.uniform(self._next(), shape, jnp.bfloat16, lo, hi)

    def permutation(self, n):
        return jax.random.permutation(self._next(), n)
kernel_name = 'parallel_sum__memory_aug_recurrent_mem_tr__dense_activation_silu__prompt'

def setup_inputs():
    _rng = _Rng(jax.random.key(int.from_bytes(__import__("os").urandom(4), "little")))
    _w = lambda a: (lambda t: t.astype(jnp.bfloat16) if jnp.issubdtype(t.dtype, jnp.floating) else t)(jnp.asarray(a))

    def _A_setup():
        B, S, Dm = (1, 2048, 448)
        H, Dh = (16, 256)
        M, seg = (8, 32)
        seg = min(seg, S)
        S = S // seg * seg
        return {'x': _w((lambda *s: _rng.normal(s) * 0.05)(B, S, Dm)), 'mem0': _w((lambda *s: _rng.normal(s) * 0.2)(B, M, Dm)), 'Wq': _w((lambda *s: _rng.normal(s) * 0.8)(Dm, H, Dh) * Dm ** (-0.5)), 'Wk': _w((lambda *s: _rng.normal(s) * 0.8)(Dm, H, Dh) * Dm ** (-0.5)), 'Wv': _w((lambda *s: _rng.normal(s) * 0.2)(Dm, H, Dh) * Dm ** (-0.5)), 'Wo': _w((lambda *s: _rng.normal(s) * 0.2)(H, Dh, Dm) * (H * Dh) ** (-0.5)), 'seg_len': seg}
    _A_in = _A_setup()

    def _B_setup():
        B, S, D, F = (1, 2048, 448, 1792)
        return {'x': _w((lambda *s: _rng.normal(s) * 0.05)(B, S, D)), 'w1': _w((lambda *s: _rng.normal(s) * 0.05)(D, F) * D ** (-0.5)), 'w2': _w((lambda *s: _rng.normal(s) * 0.05)(F, D) * F ** (-0.5))}
    _B_in = _B_setup()
    return {'A_x': _A_in['x'], 'A_mem0': _A_in['mem0'], 'A_Wq': _A_in['Wq'], 'A_Wk': _A_in['Wk'], 'A_Wv': _A_in['Wv'], 'A_Wo': _A_in['Wo'], 'A_seg_len': _A_in['seg_len'], 'B_x': _B_in['x'], 'B_w1': _B_in['w1'], 'B_w2': _B_in['w2']}

def reference(A_x, A_mem0, A_Wq, A_Wk, A_Wv, A_Wo, A_seg_len, B_x, B_w1, B_w2):

    def _A_ref(x, mem0, Wq, Wk, Wv, Wo, seg_len):
        B, S, Dm = x.shape
        H, Dh = (Wq.shape[1], Wq.shape[2])
        M = mem0.shape[1]
        scale = Dh ** (-0.5)
        n_seg = S // seg_len
        L = M + seg_len
        idx = jnp.arange(L)
        mask = (idx[:, None] < M) | (idx[:, None] >= idx[None, :])
        mem = mem0
        outs = []
        for s in range(n_seg):
            xs = x[:, s * seg_len:(s + 1) * seg_len, :].copy()
            h = jnp.concatenate([mem, xs], axis=1)
            q = jnp.einsum('btd,dhe->bhte', h, Wq)
            k = jnp.einsum('btd,dhe->bhte', h, Wk)
            v = jnp.einsum('btd,dhe->bhte', h, Wv)
            scores = jnp.einsum('bhqe,bhke->bhqk', q, k) * scale
            scores = jnp.where(mask[None, None], scores, -1000000000.0)
            p = _softmax(scores, axis=-1)
            o = jnp.einsum('bhqk,bhke->bhqe', p, v)
            o = jnp.einsum('bhte,hed->btd', o, Wo)
            mem = o[:, :M, :].copy()
            outs.append(o[:, M:, :])
        return jnp.concatenate(outs, axis=1)

    def _B_ref(x, w1, w2):
        h = jnp.einsum('bsd,df->bsf', x, w1)
        h = _silu(h)
        out = jnp.einsum('bsf,fd->bsd', h, w2)
        return out
    x = A_x
    xn = _layernorm(x, axis=-1)
    return x + _A_ref(xn, A_mem0, A_Wq, A_Wk, A_Wv, A_Wo, A_seg_len) + _B_ref(xn, B_w1, B_w2)
```

```python
import functools

import jax
import jax.numpy as jnp
from jax import lax
import jax.experimental.pallas as pl
import jax.experimental.pallas.tpu as pltpu

F32 = jnp.float32
BF16 = jnp.bfloat16
U32 = jnp.uint32
NN = (((1,), (0,)), ((), ()))
NT = (((1,), (1,)), ((), ()))
LOG2E = 1.4426950408889634

RB = 128
FC = 256
DC = 32
UNROLL = 2


def _dot(a, b, dims):
    return lax.dot_general(a, b, dims, preferred_element_type=F32)


def _layernorm(xs):
    mu = jnp.mean(xs, axis=-1, keepdims=True)
    xc = xs - mu
    var = jnp.mean(xc * xc, axis=-1, keepdims=True)
    return (xc * lax.rsqrt(var + 1e-5)).astype(BF16)


def _head_order(n_heads, l_s=1, l_p=3, l_o=5):
    out = []
    for i in range(n_heads + l_o):
        if i < n_heads:
            out.append(("Q", i))
        if 0 <= i - l_s < n_heads:
            out.append(("S", i - l_s))
        if 0 <= i - l_p < n_heads:
            out.append(("P", i - l_p))
        if 0 <= i - l_o < n_heads:
            out.append(("O", i - l_o))
    return out


def _kernel(x_hbm, mem0_hbm, wq_hbm, wk_hbm, wv_hbm, wo_hbm, w1_hbm, w2_hbm, o_hbm,
            xbuf, xnbuf, base, stage, wob, w1b, w2b, memb, wqkv, obuf,
            sem_x, sem_w, sem_misc, sem_o, *, seg):
    S, D = x_hbm.shape
    _, H, DH = wq_hbm.shape
    M = mem0_hbm.shape[0]
    Fh = w1_hbm.shape[1]
    L = M + seg
    n_seg = S // seg
    NB = S // RB
    NJ = D // DC
    PRE = NB - NJ
    NC = DH // 128
    nch = Fh // FC
    w_hbm = (wq_hbm, wk_hbm, wv_hbm)

    def x_copy(b):
        rows = pl.ds(pl.multiple_of(b * RB, RB), RB)
        return pltpu.make_async_copy(x_hbm.at[rows], xbuf.at[rows], sem_x.at[b])

    def w_copy(wi, j):
        rows = pl.ds(pl.multiple_of(j * DC, DC), DC)
        return pltpu.make_async_copy(w_hbm[wi].at[rows], stage.at[wi, rows], sem_w.at[wi, j])

    c_w1 = pltpu.make_async_copy(w1_hbm, w1b, sem_misc.at[0])
    c_w2 = pltpu.make_async_copy(w2_hbm, w2b, sem_misc.at[1])
    c_wo = pltpu.make_async_copy(wo_hbm, wob, sem_misc.at[2])
    c_mem = pltpu.make_async_copy(mem0_hbm, memb, sem_misc.at[3])

    x_copy(0).start()
    c_w1.start()
    x_copy(1).start()
    c_w2.start()
    for b in range(2, NB):
        x_copy(b).start()
    c_mem.start()
    for j in range(NJ):
        for wi in range(3):
            w_copy(wi, j).start()
    c_wo.start()

    def silu(a):
        return a * jax.nn.sigmoid(a)

    def mlp_block(b, j):
        nb = jnp.minimum(b + 1, NB - 1)
        r0 = pl.multiple_of(b * RB, RB)
        r1 = pl.multiple_of(nb * RB, RB)

        @pl.when(b + 1 < NB)
        def _():
            x_copy(nb).wait()

        if j is not None:
            for wi in range(3):
                w_copy(wi, j).wait()
        xn = xnbuf[pl.ds(r0, RB), :]
        xnbuf[pl.ds(r1, RB), :] = _layernorm(xbuf[pl.ds(r1, RB), :].astype(F32))
        y = xbuf[pl.ds(r0, RB), :].astype(F32)
        hid = [None] * nch
        for c in range(nch + 1):
            if c < nch:
                hid[c] = silu(_dot(xn, w1b[:, c * FC:(c + 1) * FC], NN)).astype(BF16)
            if c >= 1:
                y = y + _dot(hid[c - 1], w2b[(c - 1) * FC:c * FC, :], NN)
        base[pl.ds(r0, RB), :] = y
        if j is not None:
            d0 = pl.multiple_of(j * DC, DC)
            p0 = pl.multiple_of(j * (DC // 2), DC // 2)
            for wi in range(3):
                t = jnp.transpose(stage[wi, pl.ds(d0, DC)], (1, 0, 2))
                for h in range(H):
                    for c in range(NC):
                        wqkv[(h * 3 + wi) * NC + c, pl.ds(p0, DC // 2), :] = pltpu.bitcast(
                            t[h][:, c * 128:(c + 1) * 128], U32)

    x_copy(0).wait()
    xnbuf[pl.ds(0, RB), :] = _layernorm(xbuf[pl.ds(0, RB), :].astype(F32))
    c_w1.wait()
    c_w2.wait()

    def pre_body(b, carry):
        mlp_block(b, None)
        return carry

    def main_body(j, carry):
        mlp_block(j + PRE, j)
        return carry

    lax.fori_loop(0, PRE, pre_body, 0)
    lax.fori_loop(0, NJ, main_body, 0)
    c_mem.wait()
    c_wo.wait()

    row = lax.broadcasted_iota(jnp.int32, (L, L), 0)
    col = lax.broadcasted_iota(jnp.int32, (L, L), 1)
    mask = (row < M) | (row >= col)
    scale = DH ** (-0.5)
    order = _head_order(H)

    def o_copy(s):
        rows = pl.ds(pl.multiple_of(s * seg, seg), seg)
        return pltpu.make_async_copy(obuf.at[rows], o_hbm.at[rows], sem_o)

    def step(s, mem):
        r0 = pl.multiple_of(s * seg, seg)
        hcat = jnp.concatenate([mem, xnbuf[pl.ds(r0, seg), :].astype(F32)], axis=0)
        qkv = [None] * H
        e = [None] * H
        rl = [None] * H
        o = [None] * H
        acc = None
        for kind, i in order:
            if kind == "Q":
                w = jnp.concatenate(
                    [pltpu.bitcast(wqkv[i * 3 * NC + t], BF16) for t in range(3 * NC)], axis=1)
                qkv[i] = _dot(hcat, w, NN)
            elif kind == "S":
                sc = _dot(qkv[i][:, 0:DH], qkv[i][:, DH:2 * DH], NT)
                sc = jnp.where(mask, sc, -1e9 / scale)
                m = jnp.max(sc, axis=-1, keepdims=True)
                e[i] = jnp.exp2((sc - m) * (scale * LOG2E))
                l = jnp.sum(e[i], axis=-1, keepdims=True)
                r = pl.reciprocal(l, approx=True)
                rl[i] = r * (2.0 - l * r)
            elif kind == "P":
                o[i] = _dot(e[i], qkv[i][:, 2 * DH:3 * DH], NN) * rl[i]
            else:
                t = _dot(o[i], wob[i], NN)
                acc = t if acc is None else acc + t
        obuf[pl.ds(r0, seg), :] = (base[pl.ds(r0, seg), :] + acc[M:, :]).astype(BF16)
        o_copy(s).start()
        return acc[:M, :].astype(BF16).astype(F32)

    lax.fori_loop(0, n_seg, step, memb[...].astype(F32), unroll=UNROLL)
    pltpu.make_async_copy(obuf, o_hbm, sem_o).wait()


@functools.partial(jax.jit, static_argnames=("A_seg_len",))
def pallas_parallel_sum__memory_aug_recurrent_mem_tr__dense_activation_silu__prompt_kernel(
    A_x: jax.Array,
    A_mem0: jax.Array,
    A_Wq: jax.Array,
    A_Wk: jax.Array,
    A_Wv: jax.Array,
    A_Wo: jax.Array,
    A_seg_len: int,
    B_x: jax.Array,
    B_w1: jax.Array,
    B_w2: jax.Array,
):
    del B_x
    B, S, D = A_x.shape
    _, H, DH = A_Wq.shape
    M = A_mem0.shape[1]
    Fh = B_w1.shape[1]
    assert B == 1 and S % A_seg_len == 0
    any_spec = pl.BlockSpec(memory_space=pl.ANY)
    out = pl.pallas_call(
        functools.partial(_kernel, seg=A_seg_len),
        out_shape=jax.ShapeDtypeStruct((S, D), BF16),
        in_specs=[any_spec] * 8,
        out_specs=any_spec,
        scratch_shapes=[
            pltpu.VMEM((S, D), BF16),
            pltpu.VMEM((S, D), BF16),
            pltpu.VMEM((S, D), F32),
            pltpu.VMEM((3, D, H, DH), BF16),
            pltpu.VMEM((H, DH, D), BF16),
            pltpu.VMEM((D, Fh), BF16),
            pltpu.VMEM((Fh, D), BF16),
            pltpu.VMEM((M, D), BF16),
            pltpu.VMEM((H * 3 * (DH // 128), D // 2, 128), U32),
            pltpu.VMEM((S, D), BF16),
            pltpu.SemaphoreType.DMA((S // RB,)),
            pltpu.SemaphoreType.DMA((3, D // DC)),
            pltpu.SemaphoreType.DMA((4,)),
            pltpu.SemaphoreType.DMA(()),
        ],
        compiler_params=pltpu.CompilerParams(vmem_limit_bytes=100 * 1024 * 1024),
        name="rmt_mlp",
    )(A_x.reshape(S, D), A_mem0.reshape(M, D), A_Wq, A_Wk, A_Wv, A_Wo, B_w1, B_w2)
    return out.reshape(B, S, D)
```

```python
import functools
import jax
import jax.numpy as jnp
from jax import lax
import jax.experimental.pallas as pl
import jax.experimental.pallas.tpu as pltpu

F32 = jnp.float32
BF16 = jnp.bfloat16
U32 = jnp.uint32
NN = (((1,), (0,)), ((), ()))
NT = (((1,), (1,)), ((), ()))
LOG2E = 1.4426950408889634
TB = 128
DC = 32

def _dot(a, b, dims):
    return lax.dot_general(a, b, dims, preferred_element_type=F32)


def _layernorm_t(xt):
    mu = jnp.mean(xt, axis=0, keepdims=True)
    xc = xt - mu
    var = jnp.mean(xc * xc, axis=0, keepdims=True)
    return xc * lax.rsqrt(var + 1e-5)

def _head_order(n_heads, l_s=1, l_p=3, l_o=5):
    out = []
    for i in range(n_heads + l_o):
        if i < n_heads: out.append(("Q", i))
        if 0 <= i - l_s < n_heads: out.append(("S", i - l_s))
        if 0 <= i - l_p < n_heads: out.append(("P", i - l_p))
        if 0 <= i - l_o < n_heads: out.append(("O", i - l_o))
    return out

def _kernel(xt_hbm, mem0_hbm, wq_hbm, wk_hbm, wv_hbm, wot_hbm, w1_hbm, w2t_hbm, ot_hbm,
            xbuf, xnbuf, base, stage, wob, w1b, w2b, memb, wqkv, abuf, obuf,
            sem_x, sem_w, sem_misc, sem_o, *, seg, FC, lags, w2mode):
    D, S = xt_hbm.shape
    _, H, DH = wq_hbm.shape
    M = mem0_hbm.shape[0]
    Fh = w1_hbm.shape[1]
    L = M + seg
    NB = S // TB
    SPB = TB // seg
    NJ = D // DC
    PRE = NB - NJ
    NC = DH // 128
    nch = Fh // FC
    w_hbm = (wq_hbm, wk_hbm, wv_hbm)

    def x_copy(b):
        return pltpu.make_async_copy(xt_hbm.at[:, pl.ds(pl.multiple_of(b * TB, TB), TB)], xbuf.at[b], sem_x.at[b])
    def w_copy(wi, j):
        rows = pl.ds(pl.multiple_of(j * DC, DC), DC)
        return pltpu.make_async_copy(w_hbm[wi].at[rows], stage.at[wi, rows], sem_w.at[wi, j])
    def o_copy(b):
        return pltpu.make_async_copy(obuf.at[b], ot_hbm.at[:, pl.ds(pl.multiple_of(b * TB, TB), TB)], sem_o)
    c_w1 = pltpu.make_async_copy(w1_hbm, w1b, sem_misc.at[0])
    c_w2 = pltpu.make_async_copy(w2t_hbm, w2b, sem_misc.at[1])
    c_wo = pltpu.make_async_copy(wot_hbm, wob, sem_misc.at[2])
    c_mem = pltpu.make_async_copy(mem0_hbm, memb, sem_misc.at[3])

    x_copy(0).start(); c_w1.start(); x_copy(1).start(); c_w2.start()
    for b in range(2, NB): x_copy(b).start()
    c_mem.start()
    for j in range(NJ):
        for wi in range(3): w_copy(wi, j).start()
    c_wo.start()

    def silu(a):
        return a * jax.nn.sigmoid(a)

    def ln_block(b):
        xnt = _layernorm_t(xbuf[b].astype(F32))
        xnbuf[pl.ds(pl.multiple_of(b * TB, TB), TB), :] = xnt.T.astype(BF16)

    def mlp_block(b, j):
        nb = jnp.minimum(b + 1, NB - 1)
        @pl.when(b + 1 < NB)
        def _():
            x_copy(nb).wait()
        if j is not None:
            for wi in range(3): w_copy(wi, j).wait()
        xn = xnbuf[pl.ds(pl.multiple_of(b * TB, TB), TB), :]
        ln_block(nb)
        y = xbuf[b].astype(F32)
        hid = [None] * nch
        if w2mode == "chunk":
            for c in range(nch + 1):
                if c < nch:
                    hid[c] = silu(_dot(xn, w1b[:, c * FC:(c + 1) * FC], NN)).astype(BF16)
                if c >= 1:
                    y = y + _dot(w2b[:, (c - 1) * FC:c * FC], hid[c - 1], NT)
        else:
            for c in range(nch):
                hid[c] = silu(_dot(xn, w1b[:, c * FC:(c + 1) * FC], NN)).astype(BF16)
            y = y + _dot(w2b[...], jnp.concatenate(hid, axis=1), NT)
        base[b] = y
        if j is not None:
            d0 = pl.multiple_of(j * DC, DC)
            p0 = pl.multiple_of(j * (DC // 2), DC // 2)
            for wi in range(3):
                t = jnp.transpose(stage[wi, pl.ds(d0, DC)], (1, 0, 2))
                for h in range(H):
                    for c in range(NC):
                        wqkv[(h * 3 + wi) * NC + c, pl.ds(p0, DC // 2), :] = pltpu.bitcast(t[h][:, c * 128:(c + 1) * 128], U32)

    x_copy(0).wait()
    ln_block(0)
    abuf[...] = jnp.zeros(abuf.shape, F32)
    c_w1.wait(); c_w2.wait()
    def pre_body(b, carry):
        mlp_block(b, None); return carry
    def main_body(j, carry):
        mlp_block(j + PRE, j); return carry
    lax.fori_loop(0, PRE, pre_body, 0)
    lax.fori_loop(0, NJ, main_body, 0)
    c_mem.wait(); c_wo.wait()

    row = lax.broadcasted_iota(jnp.int32, (L, L), 0)
    col = lax.broadcasted_iota(jnp.int32, (L, L), 1)
    mask = (row < M) | (row >= col)
    scale = DH ** (-0.5)
    order = _head_order(H, *lags)

    def finalize(b):
        obuf[b] = (base[b] + abuf[...].T).astype(BF16)

    def step(r0, mem):
        hcat = jnp.concatenate([mem, xnbuf[pl.ds(r0, seg), :].astype(F32)], axis=0)
        qkv = [None] * H; e = [None] * H; rl = [None] * H; o = [None] * H
        acc = None
        for kind, i in order:
            if kind == "Q":
                w = jnp.concatenate([pltpu.bitcast(wqkv[i * 3 * NC + t], BF16) for t in range(3 * NC)], axis=1)
                qkv[i] = _dot(hcat, w, NN)
            elif kind == "S":
                sc = _dot(qkv[i][:, 0:DH], qkv[i][:, DH:2 * DH], NT)
                sc = jnp.where(mask, sc, -1e9 / scale)
                m = jnp.max(sc, axis=-1, keepdims=True)
                e[i] = jnp.exp2((sc - m) * (scale * LOG2E))
                l = jnp.sum(e[i], axis=-1, keepdims=True)
                r = pl.reciprocal(l, approx=True)
                rl[i] = r * (2.0 - l * r)
            elif kind == "P":
                o[i] = _dot(e[i], qkv[i][:, 2 * DH:3 * DH], NN) * rl[i]
            else:
                t = _dot(o[i], wob[i], NT)
                acc = t if acc is None else acc + t
        return acc[M:, :], acc[:M, :].astype(BF16).astype(F32)

    def block(b, mem):
        finalize(jnp.maximum(b - 1, 0))
        for k in range(SPB):
            a, mem = step(pl.multiple_of(b * TB + k * seg, seg), mem)
            abuf[pl.ds(k * seg, seg), :] = a
        @pl.when(b > 0)
        def _():
            o_copy(b - 1).start()
        return mem

    lax.fori_loop(0, NB, block, memb[...].astype(F32))
    finalize(NB - 1)
    o_copy(NB - 1).start()
    pltpu.make_async_copy(obuf, obuf, sem_o).wait()

def call(xt, mem0, wq, wk, wv, wot, w1, w2t, *, name, seg=32, FC=256, lags=(1, 3, 5), w2mode="chunk", flags=None):
    D, S = xt.shape
    _, H, DH = wq.shape
    M = mem0.shape[0]; Fh = w1.shape[1]
    NB = S // TB
    hbm = pl.BlockSpec(memory_space=pltpu.HBM)
    return pl.pallas_call(
        functools.partial(_kernel, seg=seg, FC=FC, lags=lags, w2mode=w2mode),
        out_shape=jax.ShapeDtypeStruct((D, S), BF16),
        in_specs=[hbm] * 8, out_specs=hbm,
        scratch_shapes=[
            pltpu.VMEM((NB, D, TB), BF16), pltpu.VMEM((S, D), BF16), pltpu.VMEM((NB, D, TB), F32),
            pltpu.VMEM((3, D, H, DH), BF16), pltpu.VMEM((H, D, DH), BF16),
            pltpu.VMEM((D, Fh), BF16), pltpu.VMEM((D, Fh), BF16), pltpu.VMEM((M, D), BF16),
            pltpu.VMEM((H * 3 * (DH // 128), D // 2, 128), U32), pltpu.VMEM((TB, D), F32), pltpu.VMEM((NB, D, TB), BF16),
            pltpu.SemaphoreType.DMA((NB,)), pltpu.SemaphoreType.DMA((3, D // DC)),
            pltpu.SemaphoreType.DMA((4,)), pltpu.SemaphoreType.DMA(()),
        ],
        compiler_params=pltpu.CompilerParams(vmem_limit_bytes=100 * 1024 * 1024, flags=flags or {}),
        name=name,
    )(xt, mem0, wq, wk, wv, wot, w1, w2t)


@functools.partial(jax.jit, static_argnames=("A_seg_len",))
def pallas_parallel_sum__memory_aug_recurrent_mem_tr__dense_activation_silu__prompt_kernel(
    A_x: jax.Array,
    A_mem0: jax.Array,
    A_Wq: jax.Array,
    A_Wk: jax.Array,
    A_Wv: jax.Array,
    A_Wo: jax.Array,
    A_seg_len: int,
    B_x: jax.Array,
    B_w1: jax.Array,
    B_w2: jax.Array,
):
    del B_x
    B, S, D = A_x.shape
    M = A_mem0.shape[1]
    assert B == 1 and S % A_seg_len == 0
    x_t = jnp.transpose(A_x, (0, 2, 1)).reshape(D, S)
    wo_t = jnp.transpose(A_Wo, (0, 2, 1))
    out_t = call(x_t, A_mem0.reshape(M, D), A_Wq, A_Wk, A_Wv, wo_t, B_w1, B_w2.T,
                 name="rmt_mlp", seg=A_seg_len)
    return jnp.transpose(out_t.reshape(B, D, S), (0, 2, 1))
```

```python
import functools
import jax
import jax.numpy as jnp
from jax import lax
import jax.experimental.pallas as pl
import jax.experimental.pallas.tpu as pltpu

F32 = jnp.float32
BF16 = jnp.bfloat16
U32 = jnp.uint32
NN = (((1,), (0,)), ((), ()))
NT = (((1,), (1,)), ((), ()))
LOG2E = 1.4426950408889634
TB = 128
DC = 32
FC = 256
LN = 128

def _dot(a, b, dims):
    return lax.dot_general(a, b, dims, preferred_element_type=F32)


def _layernorm_t(xt):
    mu = jnp.mean(xt, axis=0, keepdims=True)
    xc = xt - mu
    var = jnp.mean(xc * xc, axis=0, keepdims=True)
    return xc * lax.rsqrt(var + 1e-5)

def _silu(a):
    h = 0.5 * a
    return h + h * jnp.tanh(h)

def _step_order(n_heads, lag=1):
    big = [("K", i) for i in range(n_heads)] + [("U", p) for p in range(n_heads // 2)]
    out = []
    for j, b in enumerate(big):
        out.append(b)
        if 0 <= j - lag < n_heads:
            out.append(("S", j - lag))
    return out

def _kernel(xt_hbm, mem0_hbm, wq_hbm, wk_hbm, wv_hbm, wot_hbm, w1_hbm, w2t_hbm, ot_hbm,
            xbuf, xnbuf, base, stage, wob, w1b, w2b, memb, wqk, wvp, wb, abuf, obuf,
            sem_x, sem_w, sem_misc, sem_o, *, seg, H, unroll):
    D, S = xt_hbm.shape
    DH = wq_hbm.shape[1]
    M = mem0_hbm.shape[0]
    Fh = w1_hbm.shape[1]
    L = M + seg
    NB = S // TB
    SPB = TB // seg
    NJ = D // DC
    PRE = NB - NJ
    NC = DH // LN
    nch = Fh // FC
    DM = (D // LN) * LN
    DR = D - DM
    NM = DM // LN
    w_hbm = (wq_hbm, wk_hbm, wv_hbm)

    def x_copy(b):
        return pltpu.make_async_copy(xt_hbm.at[:, pl.ds(pl.multiple_of(b * TB, TB), TB)], xbuf.at[b], sem_x.at[b])
    def w_copy(wi, c, j):
        rows = pl.ds(pl.multiple_of(j * (DC * H), DC * H), DC * H)
        return pltpu.make_async_copy(w_hbm[wi].at[rows, pl.ds(c * LN, LN)], stage.at[wi * NC + c, rows], sem_w.at[wi * NC + c, j])
    def o_copy(b):
        return pltpu.make_async_copy(obuf.at[b], ot_hbm.at[:, pl.ds(pl.multiple_of(b * TB, TB), TB)], sem_o)
    c_w1 = pltpu.make_async_copy(w1_hbm, w1b, sem_misc.at[0])
    c_w2 = pltpu.make_async_copy(w2t_hbm, w2b, sem_misc.at[1])
    c_wo = pltpu.make_async_copy(wot_hbm, wob, sem_misc.at[2])
    c_mem = pltpu.make_async_copy(mem0_hbm, memb, sem_misc.at[3])
    def w_start(j):
        for wi in range(3):
            for c in range(NC): w_copy(wi, c, j).start()
    def w_wait(j):
        for wi in range(3):
            for c in range(NC): w_copy(wi, c, j).wait()

    x_copy(0).start(); c_w1.start(); x_copy(1).start(); c_w2.start()
    for b in range(2, NB): x_copy(b).start()
    c_mem.start()
    w_start(0)

    def ln_block(b):
        xnt = _layernorm_t(xbuf[b].astype(F32))
        xnbuf[pl.ds(pl.multiple_of(b * TB, TB), TB), :] = xnt.T.astype(BF16)

    def relayout(j, wi, c, part):
        r16 = pl.multiple_of((j * DC + part * 16) * H, 16 * H)
        src = stage.at[wi * NC + c, pl.ds(r16, 16 * H)].bitcast(U32)
        p0 = pl.multiple_of(j * (DC // 2) + part * 8, 8)
        for hp in range(H // 2):
            even = src[pl.ds(hp, 8, stride=H), :]
            odd = src[pl.ds(hp + H // 2, 8, stride=H), :]
            lo = (even & U32(0xFFFF)) | (odd << 16)
            hi = (even >> 16) | (odd & U32(0xFFFF0000))
            for k, val in enumerate((lo, hi)):
                h = 2 * hp + k
                if wi < 2:
                    wqk[(h * 2 + wi) * NC + c, pl.ds(p0, 8), :] = val
                else:
                    wvp[h * NC + c, pl.ds(p0, 8), :] = val

    def mlp_block(b, j):
        nb = jnp.minimum(b + 1, NB - 1)
        @pl.when(b + 1 < NB)
        def _():
            x_copy(nb).wait()
        @pl.when(b + 1 < NJ)
        def _():
            w_start(b + 1)
        @pl.when(b + 1 == NJ)
        def _():
            c_wo.start()
        if j is not None:
            w_wait(j)
        xn = xnbuf[pl.ds(pl.multiple_of(b * TB, TB), TB), :]
        ln_block(nb)
        pieces = [] if j is None else [(wi, c, part) for wi in range(3) for part in range(DC // 16) for c in range(NC)]
        hid = []
        for c in range(nch):
            hid.append(_silu(_dot(xn, w1b[:, c * FC:(c + 1) * FC], NN)).astype(BF16))
            for q in range((len(pieces) * c) // nch, (len(pieces) * (c + 1)) // nch):
                relayout(j, *pieces[q])
        base[b] = xbuf[b].astype(F32) + _dot(w2b[...], jnp.concatenate(hid, axis=1), NT)

    with jax.named_scope("startup"):
        x_copy(0).wait()
        ln_block(0)
        abuf[...] = jnp.zeros(abuf.shape, F32)
        c_w1.wait()
        c_w2.wait()
    def pre_body(b, carry):
        mlp_block(b, None); return carry
    def main_body(j, carry):
        mlp_block(j + PRE, j); return carry
    with jax.named_scope("pre"):
        lax.fori_loop(0, PRE, pre_body, 0)
    with jax.named_scope("main"):
        lax.fori_loop(0, NJ, main_body, 0)
    with jax.named_scope("waitwo"):
        c_mem.wait(); c_wo.wait()

    def fold_pair(p, carry):
        bs = []
        for k in range(2):
            h = 2 * p + k
            wv_h = jnp.concatenate([pltpu.bitcast(wvp[h * NC + c], BF16) for c in range(NC)], axis=1)
            bs.append(_dot(wv_h, wob[h], NT).astype(BF16))
        tiles = [bs[0][:, t * LN:(t + 1) * LN] for t in range(NM)]
        tiles.append(jnp.concatenate([bs[0][:, DM:], bs[1][:, DM:]], axis=1))
        tiles += [bs[1][:, t * LN:(t + 1) * LN] for t in range(NM)]
        for t, tile in enumerate(tiles):
            wb[p * (2 * NM + 1) + t] = pltpu.bitcast(tile, U32)
        return carry
    with jax.named_scope("fold"):
        lax.fori_loop(0, H // 2, fold_pair, 0)

    row = lax.broadcasted_iota(jnp.int32, (L, L), 0)
    col = lax.broadcasted_iota(jnp.int32, (L, L), 1)
    mask = (row < M) | (row >= col)
    lo_half = lax.broadcasted_iota(jnp.int32, (L, LN), 1) < DR
    scale = DH ** (-0.5)
    order = _step_order(H)
    hpg = LN // L
    groups = [list(range(g, min(g + hpg, H))) for g in range(0, H, hpg)]
    TP = 2 * NM + 1

    def finalize(b):
        obuf[b] = (base[b] + abuf[...].T).astype(BF16)

    def step(r0, mem):
        hcat = jnp.concatenate([mem, xnbuf[pl.ds(r0, seg), :].astype(F32)], axis=0)
        qk = [None] * H; p = [None] * H; u = [None] * (H // 2)
        for kind, i in order:
            if kind == "K":
                w = jnp.concatenate([pltpu.bitcast(wqk[i * 2 * NC + t], BF16) for t in range(2 * NC)], axis=1)
                qk[i] = _dot(hcat, w, NN)
            elif kind == "S":
                sc = _dot(qk[i][:, 0:DH], qk[i][:, DH:2 * DH], NT)
                sc = jnp.where(mask, sc, -1e9 / scale)
                m = jnp.max(sc, axis=-1, keepdims=True)
                e = jnp.exp2((sc - m) * (scale * LOG2E))
                l = jnp.sum(e, axis=-1, keepdims=True)
                r = pl.reciprocal(l, approx=True)
                p[i] = e * (r * (2.0 - l * r))
            else:
                w = jnp.concatenate([pltpu.bitcast(wb[i * TP + t], BF16) for t in range(TP)], axis=1)
                u[i] = _dot(hcat, w, NN)
        acc = None
        for hs in groups:
            npad = LN - L * len(hs)
            rows = []
            for h in hs:
                up = u[h // 2]
                rem = up[:, DM:DM + LN]
                if h % 2 == 0:
                    rows.append(jnp.concatenate([up[:, 0:DM], jnp.where(lo_half, rem, 0.0)], axis=1))
                else:
                    rows.append(jnp.concatenate([up[:, DM + LN:], jnp.where(lo_half, 0.0, rem)], axis=1))
            pg = jnp.concatenate([p[h] for h in hs] + [jnp.zeros((L, npad), F32)], axis=1)
            ug = jnp.concatenate(rows + [jnp.zeros((npad, DM + LN), F32)], axis=0).astype(BF16)
            t = _dot(pg, ug, NN)
            acc = t if acc is None else acc + t
        rem = acc[:, DM:]
        rem = rem + pltpu.roll(rem, DR, 1)
        out = jnp.concatenate([acc[:, :DM], rem[:, :DR]], axis=1)
        return out[M:, :], out[:M, :].astype(BF16).astype(F32)

    def block(b, mem):
        finalize(jnp.maximum(b - 1, 0))
        if unroll == SPB:
            for k in range(SPB):
                a, mem = step(pl.multiple_of(b * TB + k * seg, seg), mem)
                abuf[pl.ds(k * seg, seg), :] = a
        else:
            def inner(k, mem):
                a, mem2 = step(pl.multiple_of(b * TB + k * seg, seg), mem)
                abuf[pl.ds(pl.multiple_of(k * seg, seg), seg), :] = a
                return mem2
            mem = lax.fori_loop(0, SPB, inner, mem, unroll=unroll)
        @pl.when(b > 0)
        def _():
            o_copy(b - 1).start()
        return mem

    with jax.named_scope("steps"):
        lax.fori_loop(0, NB, block, memb[...].astype(F32))
    with jax.named_scope("epilogue"):
        finalize(NB - 1)
        o_copy(NB - 1).start()
        pltpu.make_async_copy(obuf, obuf, sem_o).wait()

def call(xt, mem0, wq, wk, wv, wot, w1, w2t, *, name, seg=32, unroll=4):
    D, S = xt.shape
    H, _, DH = wot.shape
    M = mem0.shape[0]; Fh = w1.shape[1]
    NB = S // TB
    NC = DH // LN
    hbm = pl.BlockSpec(memory_space=pltpu.HBM)
    return pl.pallas_call(
        functools.partial(_kernel, seg=seg, H=H, unroll=unroll),
        out_shape=jax.ShapeDtypeStruct((D, S), BF16),
        in_specs=[hbm] * 8, out_specs=hbm,
        scratch_shapes=[
            pltpu.VMEM((NB, D, TB), BF16), pltpu.VMEM((S, D), BF16), pltpu.VMEM((NB, D, TB), F32),
            pltpu.VMEM((3 * NC, D * H, LN), BF16), pltpu.VMEM((H, D, DH), BF16),
            pltpu.VMEM((D, Fh), BF16), pltpu.VMEM((D, Fh), BF16), pltpu.VMEM((M, D), BF16),
            pltpu.VMEM((H * 2 * NC, D // 2, LN), U32), pltpu.VMEM((H * NC, D // 2, LN), U32),
            pltpu.VMEM(((H // 2) * (2 * (D // LN) + 1), D // 2, LN), U32),
            pltpu.VMEM((TB, D), F32), pltpu.VMEM((NB, D, TB), BF16),
            pltpu.SemaphoreType.DMA((NB,)), pltpu.SemaphoreType.DMA((3 * NC, D // DC)),
            pltpu.SemaphoreType.DMA((4,)), pltpu.SemaphoreType.DMA(()),
        ],
        compiler_params=pltpu.CompilerParams(vmem_limit_bytes=100 * 1024 * 1024),
        name=name,
    )(xt, mem0, wq.reshape(D * H, DH), wk.reshape(D * H, DH), wv.reshape(D * H, DH), wot, w1, w2t)


@functools.partial(jax.jit, static_argnames=("A_seg_len",))
def pallas_parallel_sum__memory_aug_recurrent_mem_tr__dense_activation_silu__prompt_kernel(
    A_x: jax.Array,
    A_mem0: jax.Array,
    A_Wq: jax.Array,
    A_Wk: jax.Array,
    A_Wv: jax.Array,
    A_Wo: jax.Array,
    A_seg_len: int,
    B_x: jax.Array,
    B_w1: jax.Array,
    B_w2: jax.Array,
):
    del B_x
    B, S, D = A_x.shape
    M = A_mem0.shape[1]
    assert B == 1 and S % A_seg_len == 0
    x_t = jnp.transpose(A_x, (0, 2, 1)).reshape(D, S)
    wo_t = jnp.transpose(A_Wo, (0, 2, 1))
    out_t = call(x_t, A_mem0.reshape(M, D), A_Wq, A_Wk, A_Wv, wo_t, B_w1, B_w2.T,
                 name="rmt_mlp", seg=A_seg_len)
    return jnp.transpose(out_t.reshape(B, D, S), (0, 2, 1))
```

```python
import functools
import jax
import jax.numpy as jnp
from jax import lax
import jax.experimental.pallas as pl
import jax.experimental.pallas.tpu as pltpu

F32 = jnp.float32
BF16 = jnp.bfloat16
U32 = jnp.uint32
NN = (((1,), (0,)), ((), ()))
NT = (((1,), (1,)), ((), ()))
LOG2E = 1.4426950408889634
TB = 128
GB = 2
DC = 32
FC = 256
LN = 128

def _dot(a, b, dims):
    return lax.dot_general(a, b, dims, preferred_element_type=F32)


def _layernorm_t(xt):
    mu = jnp.mean(xt, axis=0, keepdims=True)
    xc = xt - mu
    var = jnp.mean(xc * xc, axis=0, keepdims=True)
    return xc * lax.rsqrt(var + 1e-5)

def _silu(a):
    h = 0.5 * a
    return h + h * jnp.tanh(h)

def _step_order(n_heads, lag=1):
    big = [("K", i) for i in range(n_heads)] + [("U", p) for p in range(n_heads // 2)]
    out = []
    for j, b in enumerate(big):
        out.append(b)
        if 0 <= j - lag < n_heads:
            out.append(("S", j - lag))
    return out

def _kernel(xt_hbm, mem0_hbm, wq_hbm, wk_hbm, wv_hbm, wot_hbm, w1_hbm, w2t_hbm, ot_hbm,
            xbuf, xnbuf, base, stage, wob, w1b, w2b, memb, wqk, wvp, wb, abuf, obuf,
            sem_x, sem_w, sem_misc, sem_o, *, seg, H, unroll, dmapos):
    D, S = xt_hbm.shape
    DH = wq_hbm.shape[1]
    M = mem0_hbm.shape[0]
    Fh = w1_hbm.shape[1]
    L = M + seg
    NB = S // TB
    SPB = TB // seg
    NJ = D // DC
    PRE = NB - NJ
    NC = DH // LN
    nch = Fh // FC
    DM = (D // LN) * LN
    DR = D - DM
    NM = DM // LN
    w_hbm = (wq_hbm, wk_hbm, wv_hbm)

    def x_copy(b):
        return pltpu.make_async_copy(xt_hbm.at[:, pl.ds(pl.multiple_of(b * TB, TB), TB)], xbuf.at[b], sem_x.at[b])
    def w_copy(wi, c, j):
        rows = pl.ds(pl.multiple_of(j * (GB * DC * H), GB * DC * H), GB * DC * H)
        return pltpu.make_async_copy(w_hbm[wi].at[rows, pl.ds(c * LN, LN)], stage.at[wi * NC + c, rows], sem_w.at[wi * NC + c, j])
    def o_copy(b):
        return pltpu.make_async_copy(obuf.at[b], ot_hbm.at[:, pl.ds(pl.multiple_of(b * TB, TB), TB)], sem_o)
    c_w1 = pltpu.make_async_copy(w1_hbm, w1b, sem_misc.at[0])
    c_w2 = pltpu.make_async_copy(w2t_hbm, w2b, sem_misc.at[1])
    c_wo = pltpu.make_async_copy(wot_hbm, wob, sem_misc.at[2])
    c_mem = pltpu.make_async_copy(mem0_hbm, memb, sem_misc.at[3])
    def w_start(j):
        for wi in range(3):
            for c in range(NC): w_copy(wi, c, j).start()
    def w_wait(j):
        for wi in range(3):
            for c in range(NC): w_copy(wi, c, j).wait()

    def issue_seq(starts):
        def body(i, carry):
            for k, st in enumerate(starts):
                pl.when(i == k)(st)
            return carry
        lax.fori_loop(0, len(starts), body, 0)
    x_copy(0).start()
    c_w1.start()
    lax.fori_loop(1, 2, lambda b, c: (x_copy(b).start(), c_w2.start(), c)[-1], 0)
    lax.fori_loop(2, NB, lambda b, c: (x_copy(b).start(), c)[-1], 0)
    c_mem.start()
    lax.fori_loop(0, 2, lambda g, c: (w_start(g), c)[-1], 0)

    def ln_block(b):
        xnt = _layernorm_t(xbuf[b].astype(F32))
        xnbuf[pl.ds(pl.multiple_of(b * TB, TB), TB), :] = xnt.T.astype(BF16)

    def relayout(j, wi, c, part):
        r16 = pl.multiple_of((j * DC + part * 16) * H, 16 * H)
        src = stage.at[wi * NC + c, pl.ds(r16, 16 * H)].bitcast(U32)
        p0 = pl.multiple_of(j * (DC // 2) + part * 8, 8)
        for hp in range(H // 2):
            even = src[pl.ds(hp, 8, stride=H), :]
            odd = src[pl.ds(hp + H // 2, 8, stride=H), :]
            lo = (even & U32(0xFFFF)) | (odd << 16)
            hi = (even >> 16) | (odd & U32(0xFFFF0000))
            for k, val in enumerate((lo, hi)):
                h = 2 * hp + k
                if wi < 2:
                    wqk[(h * 2 + wi) * NC + c, pl.ds(p0, 8), :] = val
                else:
                    wvp[h * NC + c, pl.ds(p0, 8), :] = val

    def mlp_block(b, j):
        nb = jnp.minimum(b + 1, NB - 1)
        xn = xnbuf[pl.ds(pl.multiple_of(b * TB, TB), TB), :]
        ln_block(nb)
        pieces = [] if j is None else [(wi, c, part) for wi in range(3) for part in range(DC // 16) for c in range(NC)]
        hid = []
        for c in range(nch):
            hid.append(_silu(_dot(xn, w1b[:, c * FC:(c + 1) * FC], NN)).astype(BF16))
            for q in range((len(pieces) * c) // nch, (len(pieces) * (c + 1)) // nch):
                relayout(j, *pieces[q])
        base[b] = xbuf[b].astype(F32) + _dot(w2b[...], jnp.concatenate(hid, axis=1), NT)

    with jax.named_scope("st_x0"):
        x_copy(0).wait()
    with jax.named_scope("st_ln0"):
        ln_block(0)
        abuf[...] = jnp.zeros(abuf.shape, F32)
    with jax.named_scope("st_w1"):
        x_copy(1).wait()
        c_w1.wait()
    with jax.named_scope("st_w2"):
        c_w2.wait()
    def pre_body(b, carry):
        mlp_block(b, None); return carry
    def main_body(j, carry):
        mlp_block(j + PRE, j); return carry
    with jax.named_scope("pre"):
        for b in range(2, PRE + 1): x_copy(b).wait()
        lax.fori_loop(0, PRE, pre_body, 0)
    NG = NJ // GB
    def group_body(g, carry):
        w_wait(g)
        @pl.when(g + 2 < NG)
        def _():
            w_start(g + 2)
        @pl.when(g + 2 == NG)
        def _():
            c_wo.start()
        for k in range(GB):
            b = PRE + g * GB + k + 1
            @pl.when(b < NB)
            def _():
                x_copy(jnp.minimum(b, NB - 1)).wait()
        lax.fori_loop(g * GB, (g + 1) * GB, main_body, 0)
        return carry
    with jax.named_scope("main"):
        lax.fori_loop(0, NG, group_body, 0)
    with jax.named_scope("waitwo"):
        c_mem.wait(); c_wo.wait()

    def fold_pair(p, carry):
        bs = []
        for k in range(2):
            h = 2 * p + k
            wv_h = jnp.concatenate([pltpu.bitcast(wvp[h * NC + c], BF16) for c in range(NC)], axis=1)
            bs.append(_dot(wv_h, wob[h], NT).astype(BF16))
        tiles = [bs[0][:, t * LN:(t + 1) * LN] for t in range(NM)]
        tiles.append(jnp.concatenate([bs[0][:, DM:], bs[1][:, DM:]], axis=1))
        tiles += [bs[1][:, t * LN:(t + 1) * LN] for t in range(NM)]
        for t, tile in enumerate(tiles):
            wb[p * (2 * NM + 1) + t] = pltpu.bitcast(tile, U32)
        return carry
    with jax.named_scope("fold"):
        lax.fori_loop(0, H // 2, fold_pair, 0)

    row = lax.broadcasted_iota(jnp.int32, (L, L), 0)
    col = lax.broadcasted_iota(jnp.int32, (L, L), 1)
    mask = (row < M) | (row >= col)
    lo_half = lax.broadcasted_iota(jnp.int32, (L, LN), 1) < DR
    scale = DH ** (-0.5)
    order = _step_order(H)
    hpg = LN // L
    groups = [list(range(g, min(g + hpg, H))) for g in range(0, H, hpg)]
    TP = 2 * NM + 1

    def finalize(b):
        obuf[b] = (base[b] + abuf[...].T).astype(BF16)

    def step(r0, mem):
        hcat = jnp.concatenate([mem, xnbuf[pl.ds(r0, seg), :].astype(F32)], axis=0)
        qk = [None] * H; p = [None] * H; u = [None] * (H // 2)
        for kind, i in order:
            if kind == "K":
                w = jnp.concatenate([pltpu.bitcast(wqk[i * 2 * NC + t], BF16) for t in range(2 * NC)], axis=1)
                qk[i] = _dot(hcat, w, NN)
            elif kind == "S":
                sc = _dot(qk[i][:, 0:DH], qk[i][:, DH:2 * DH], NT)
                sc = jnp.where(mask, sc, -1e9 / scale)
                m = jnp.max(sc, axis=-1, keepdims=True)
                e = jnp.exp2((sc - m) * (scale * LOG2E))
                l = jnp.sum(e, axis=-1, keepdims=True)
                r = pl.reciprocal(l, approx=True)
                p[i] = e * (r * (2.0 - l * r))
            else:
                w = jnp.concatenate([pltpu.bitcast(wb[i * TP + t], BF16) for t in range(TP)], axis=1)
                u[i] = _dot(hcat, w, NN)
        acc = None
        for hs in groups:
            npad = LN - L * len(hs)
            rows = []
            for h in hs:
                up = u[h // 2]
                rem = up[:, DM:DM + LN]
                if h % 2 == 0:
                    rows.append(jnp.concatenate([up[:, 0:DM], jnp.where(lo_half, rem, 0.0)], axis=1))
                else:
                    rows.append(jnp.concatenate([up[:, DM + LN:], jnp.where(lo_half, 0.0, rem)], axis=1))
            pg = jnp.concatenate([p[h] for h in hs] + [jnp.zeros((L, npad), F32)], axis=1)
            ug = jnp.concatenate(rows + [jnp.zeros((npad, DM + LN), F32)], axis=0).astype(BF16)
            t = _dot(pg, ug, NN)
            acc = t if acc is None else acc + t
        rem = acc[:, DM:]
        rem = rem + pltpu.roll(rem, DR, 1)
        out = jnp.concatenate([acc[:, :DM], rem[:, :DR]], axis=1)
        return out[M:, :], out[:M, :].astype(BF16).astype(F32)

    def block(b, mem):
        finalize(jnp.maximum(b - 1, 0))
        if unroll == SPB:
            for k in range(SPB):
                a, mem = step(pl.multiple_of(b * TB + k * seg, seg), mem)
                abuf[pl.ds(k * seg, seg), :] = a
        else:
            def inner(k, mem):
                a, mem2 = step(pl.multiple_of(b * TB + k * seg, seg), mem)
                abuf[pl.ds(pl.multiple_of(k * seg, seg), seg), :] = a
                return mem2
            mem = lax.fori_loop(0, SPB, inner, mem, unroll=unroll)
        @pl.when(b > 0)
        def _():
            o_copy(b - 1).start()
        return mem

    with jax.named_scope("steps"):
        lax.fori_loop(0, NB, block, memb[...].astype(F32))
    with jax.named_scope("epilogue"):
        finalize(NB - 1)
        o_copy(NB - 1).start()
        pltpu.make_async_copy(obuf, obuf, sem_o).wait()

def call(xt, mem0, wq, wk, wv, wot, w1, w2t, *, name, seg=32, unroll=4, nobc=True, dmapos=0):
    D, S = xt.shape
    H, _, DH = wot.shape
    M = mem0.shape[0]; Fh = w1.shape[1]
    NB = S // TB
    NC = DH // LN
    hbm = pl.BlockSpec(memory_space=pltpu.HBM)
    return pl.pallas_call(
        functools.partial(_kernel, seg=seg, H=H, unroll=unroll, dmapos=dmapos),
        out_shape=jax.ShapeDtypeStruct((D, S), BF16),
        in_specs=[hbm] * 8, out_specs=hbm,
        scratch_shapes=[
            pltpu.VMEM((NB, D, TB), BF16), pltpu.VMEM((S, D), BF16), pltpu.VMEM((NB, D, TB), F32),
            pltpu.VMEM((3 * NC, D * H, LN), BF16), pltpu.VMEM((H, D, DH), BF16),
            pltpu.VMEM((D, Fh), BF16), pltpu.VMEM((D, Fh), BF16), pltpu.VMEM((M, D), BF16),
            pltpu.VMEM((H * 2 * NC, D // 2, LN), U32), pltpu.VMEM((H * NC, D // 2, LN), U32),
            pltpu.VMEM(((H // 2) * (2 * (D // LN) + 1), D // 2, LN), U32),
            pltpu.VMEM((TB, D), F32), pltpu.VMEM((NB, D, TB), BF16),
            pltpu.SemaphoreType.DMA((NB,)), pltpu.SemaphoreType.DMA((3 * NC, D // (DC * GB))),
            pltpu.SemaphoreType.DMA((4,)), pltpu.SemaphoreType.DMA(()),
        ],
        compiler_params=pltpu.CompilerParams(vmem_limit_bytes=100 * 1024 * 1024, disable_bounds_checks=nobc),
        name=name,
    )(xt, mem0, wq.reshape(D * H, DH), wk.reshape(D * H, DH), wv.reshape(D * H, DH), wot, w1, w2t)


@functools.partial(jax.jit, static_argnames=("A_seg_len",))
def pallas_parallel_sum__memory_aug_recurrent_mem_tr__dense_activation_silu__prompt_kernel(
    A_x: jax.Array,
    A_mem0: jax.Array,
    A_Wq: jax.Array,
    A_Wk: jax.Array,
    A_Wv: jax.Array,
    A_Wo: jax.Array,
    A_seg_len: int,
    B_x: jax.Array,
    B_w1: jax.Array,
    B_w2: jax.Array,
):
    del B_x
    B, S, D = A_x.shape
    M = A_mem0.shape[1]
    assert B == 1 and S % A_seg_len == 0
    x_t = jnp.transpose(A_x, (0, 2, 1)).reshape(D, S)
    wo_t = jnp.transpose(A_Wo, (0, 2, 1))
    out_t = call(x_t, A_mem0.reshape(M, D), A_Wq, A_Wk, A_Wv, wo_t, B_w1, B_w2.T,
                 name="rmt_mlp", seg=A_seg_len)
    return jnp.transpose(out_t.reshape(B, D, S), (0, 2, 1))
```

```python
import functools
import jax
import jax.numpy as jnp
from jax import lax
import jax.experimental.pallas as pl
import jax.experimental.pallas.tpu as pltpu

F32 = jnp.float32
BF16 = jnp.bfloat16
U32 = jnp.uint32
NN = (((1,), (0,)), ((), ()))
NT = (((1,), (1,)), ((), ()))
LOG2E = 1.4426950408889634
TB = 128
GB = 2
DC = 32
FC = 256
LN = 128

def _dot(a, b, dims):
    return lax.dot_general(a, b, dims, preferred_element_type=F32)


def _layernorm_t(xt):
    mu = jnp.mean(xt, axis=0, keepdims=True)
    xc = xt - mu
    var = jnp.mean(xc * xc, axis=0, keepdims=True)
    return xc * lax.rsqrt(var + 1e-5)

def _silu(a):
    h = 0.5 * a
    return h + h * jnp.tanh(h)

def _step_order(n_heads, lag=1):
    big = [("K", i) for i in range(n_heads)] + [("U", p) for p in range(n_heads // 2)]
    out = []
    for j, b in enumerate(big):
        out.append(b)
        if 0 <= j - lag < n_heads:
            out.append(("S", j - lag))
    return out

def _kernel(xt_hbm, mem0_hbm, wq_hbm, wk_hbm, wv_hbm, wot_hbm, w1_hbm, w2t_hbm, ot_hbm,
            xbuf, xnbuf, base, hidb, stage, wob, w1b, w2b, memb, wqk, wvp, wb, abuf, obuf,
            sem_x, sem_w, sem_misc, sem_o, *, seg, H, unroll, dmapos, memlast, vdense, roundmem, lag, mainunroll, foldunroll, blockunroll):
    D, S = xt_hbm.shape
    DH = wq_hbm.shape[1]
    M = mem0_hbm.shape[0]
    Fh = w1_hbm.shape[1]
    L = M + seg
    NB = S // TB
    SPB = TB // seg
    NJ = D // DC
    PRE = NB - NJ
    NC = DH // LN
    nch = Fh // FC
    DM = (D // LN) * LN
    DR = D - DM
    NM = DM // LN
    DP = DM + LN
    w_hbm = (wq_hbm, wk_hbm, wv_hbm)

    def x_copy(b):
        return pltpu.make_async_copy(xt_hbm.at[:, pl.ds(pl.multiple_of(b * TB, TB), TB)], xbuf.at[b], sem_x.at[b])
    def w_copy(wi, c, j):
        rows = pl.ds(pl.multiple_of(j * (GB * DC * H), GB * DC * H), GB * DC * H)
        return pltpu.make_async_copy(w_hbm[wi].at[rows, pl.ds(c * LN, LN)], stage.at[wi * NC + c, rows], sem_w.at[wi * NC + c, j])
    def o_copy(b):
        return pltpu.make_async_copy(obuf.at[b], ot_hbm.at[:, pl.ds(pl.multiple_of(b * TB, TB), TB)], sem_o)
    c_w1 = pltpu.make_async_copy(w1_hbm, w1b, sem_misc.at[0])
    c_w2 = pltpu.make_async_copy(w2t_hbm, w2b, sem_misc.at[1])
    c_wo = pltpu.make_async_copy(wot_hbm, wob, sem_misc.at[2])
    c_mem = pltpu.make_async_copy(mem0_hbm, memb, sem_misc.at[3])
    def w_start(j):
        for wi in range(3):
            for c in range(NC): w_copy(wi, c, j).start()
    def w_wait(j):
        for wi in range(3):
            for c in range(NC): w_copy(wi, c, j).wait()

    def issue_seq(starts):
        def body(i, carry):
            for k, st in enumerate(starts):
                pl.when(i == k)(st)
            return carry
        lax.fori_loop(0, len(starts), body, 0)
    x_copy(0).start()
    c_w1.start()
    lax.fori_loop(1, PRE + 1, lambda b, c: (x_copy(b).start(), c)[-1], 0)
    c_w2.start()
    def first_groups(g, c):
        for k in range(GB):
            x_copy(PRE + 1 + g * GB + k).start()
        w_start(g)
        return c
    lax.fori_loop(0, 2, first_groups, 0)
    lax.fori_loop(PRE + 1 + 2 * GB, NB, lambda b, c: (x_copy(b).start(), c)[-1], 0)
    c_mem.start()

    def ln_block(b):
        xnt = _layernorm_t(xbuf[b].astype(F32))
        xnt = jnp.concatenate([xnt, jnp.zeros((DP - D, TB), F32)], axis=0)
        xnbuf[pl.ds(pl.multiple_of(b * TB, TB), TB), :] = xnt.T.astype(BF16)

    def relayout(j, wi, c, part, dup):
        r16 = pl.multiple_of((j * DC + part * 16) * H, 16 * H)
        src = stage.at[wi * NC + c, pl.ds(r16, 16 * H)].bitcast(U32)
        p0 = pl.multiple_of(j * (DC // 2) + part * 8, 8)
        for hp in range(H // 2):
            even = src[pl.ds(hp, 8, stride=H), :]
            odd = src[pl.ds(hp + H // 2, 8, stride=H), :]
            lo = (even & U32(0xFFFF)) | (odd << 16)
            hi = (even >> 16) | (odd & U32(0xFFFF0000))
            for k, val in enumerate((lo, hi)):
                h = 2 * hp + k
                if wi < 2:
                    wqk[(h * 2 + wi) * NC + c, pl.ds(p0, 8), :] = val
                    if dup:
                        wqk[(h * 2 + wi) * NC + c, pl.ds(p0 + DR // 2, 8), :] = val
                else:
                    wvp[h * NC + c, pl.ds(p0, 8), :] = val

    def mlp_up(b, j, dup=False):
        nb = jnp.minimum(b + 1, NB - 1)
        xn = xnbuf[pl.ds(pl.multiple_of(b * TB, TB), TB), :D]
        ln_block(nb)
        pieces = [] if j is None else [(wi, c, part) for wi in range(3) for part in range(DC // 16) for c in range(NC)]
        hid = []
        for c in range(nch):
            hid.append(_silu(_dot(xn, w1b[:, c * FC:(c + 1) * FC], NN)).astype(BF16))
            for q in range((len(pieces) * c) // nch, (len(pieces) * (c + 1)) // nch):
                relayout(j, *pieces[q], dup)
        return jnp.concatenate(hid, axis=1)

    def mlp_down(b, hid):
        base[b] = xbuf[b].astype(F32) + _dot(w2b[...], hid, NT)

    def mlp_block(b, j, dup=False):
        mlp_down(b, mlp_up(b, j, dup))

    with jax.named_scope("st_x0"):
        x_copy(0).wait()
    with jax.named_scope("st_ln0"):
        ln_block(0)
        abuf[...] = jnp.zeros(abuf.shape, F32)
    with jax.named_scope("st_w1"):
        x_copy(1).wait()
        c_w1.wait()
    def main_body(j, carry):
        mlp_block(j + PRE, j); return carry
    with jax.named_scope("pre_up"):
        for b in range(2, PRE + 1): x_copy(b).wait()
        for b in range(PRE):
            hidb[b] = mlp_up(b, None)
    with jax.named_scope("st_w2"):
        c_w2.wait()
    with jax.named_scope("pre_down"):
        for b in range(PRE):
            mlp_down(b, hidb[b])
    NG = NJ // GB
    def group_body(g, carry, dup=False):
        w_wait(g)
        @pl.when(g + 2 < NG)
        def _():
            w_start(g + 2)
        @pl.when(g + 2 == NG)
        def _():
            c_wo.start()
        for k in range(GB):
            b = PRE + g * GB + k + 1
            @pl.when(b < NB)
            def _():
                x_copy(jnp.minimum(b, NB - 1)).wait()
        lax.fori_loop(g * GB, (g + 1) * GB, lambda j, c: (mlp_block(j + PRE, j, dup), c)[-1], 0)
        return carry
    assert (NG - 1) * GB * DC == DM and GB * DC == DR
    with jax.named_scope("main"):
        lax.fori_loop(0, NG - 1, group_body, 0)
        group_body(NG - 1, 0, True)
    with jax.named_scope("waitwo"):
        c_mem.wait(); c_wo.wait()

    def fold_pair(p, carry):
        bs = []
        for k in range(2):
            h = 2 * p + k
            wv_h = jnp.concatenate([pltpu.bitcast(wvp[h * NC + c], BF16) for c in range(NC)], axis=1)
            bs.append(_dot(wv_h, wob[h], NT).astype(BF16))
        tiles = [bs[0][:, t * LN:(t + 1) * LN] for t in range(NM)]
        tiles.append(jnp.concatenate([bs[0][:, DM:], bs[1][:, DM:]], axis=1))
        tiles += [bs[1][:, t * LN:(t + 1) * LN] for t in range(NM)]
        for t, tile in enumerate(tiles):
            packed = pltpu.bitcast(tile, U32)
            wb[p * (2 * NM + 1) + t, pl.ds(0, D // 2), :] = packed
            wb[p * (2 * NM + 1) + t, pl.ds(D // 2, DR // 2), :] = packed[DM // 2:, :]
        return carry
    with jax.named_scope("fold"):
        lax.fori_loop(0, H // 2, fold_pair, 0, unroll=foldunroll)

    row = lax.broadcasted_iota(jnp.int32, (L, L), 0)
    col = lax.broadcasted_iota(jnp.int32, (L, L), 1)
    if memlast:
        mask = (row >= seg) | (col >= seg) | (row >= col)
    else:
        mask = (row < M) | (row >= col)
    lo_half = lax.broadcasted_iota(jnp.int32, (L, LN), 1) < DR
    scale = DH ** (-0.5)
    order = _step_order(H, lag)
    hpg = LN // L
    groups = [list(range(g, min(g + hpg, H))) for g in range(0, H, hpg)]
    TP = 2 * NM + 1

    def finalize(b):
        a = abuf[...]
        rem = a[:, DM:]
        rem = rem + pltpu.roll(rem, DR, 1)
        at = jnp.concatenate([a[:, :DM].T, rem.T[:DR]], axis=0)
        obuf[b] = (base[b] + at).astype(BF16)

    def step(r0, mem):
        xs = xnbuf[pl.ds(r0, seg), :].astype(F32)
        hcat = jnp.concatenate([xs, mem] if memlast else [mem, xs], axis=0)
        qk = [None] * H; p = [None] * H; u = [None] * (H // 2)
        for kind, i in order:
            if kind == "K":
                w = jnp.concatenate([pltpu.bitcast(wqk[i * 2 * NC + t], BF16) for t in range(2 * NC)], axis=1)
                qk[i] = _dot(hcat, w, NN)
            elif kind == "S":
                sc = _dot(qk[i][:, 0:DH], qk[i][:, DH:2 * DH], NT)
                sc = jnp.where(mask, sc, -1e9 / scale)
                m = jnp.max(sc, axis=-1, keepdims=True)
                e = jnp.exp2((sc - m) * (scale * LOG2E))
                l = jnp.sum(e, axis=-1, keepdims=True)
                r = pl.reciprocal(l, approx=True)
                p[i] = e * (r * (2.0 - l * r))
            else:
                w = jnp.concatenate([pltpu.bitcast(wb[i * TP + t], BF16) for t in range(TP)], axis=1)
                u[i] = _dot(hcat, w, NN)
        def urows(h):
            up = u[h // 2]
            rem = up[:, DM:DM + LN]
            if h % 2 == 0:
                return jnp.concatenate([up[:, 0:DM], jnp.where(lo_half, rem, 0.0)], axis=1)
            return jnp.concatenate([up[:, DM + LN:], jnp.where(lo_half, 0.0, rem)], axis=1)
        def memfirst(a):
            return jnp.concatenate([a[seg:], a[:seg]], axis=0) if memlast else a
        acc = None
        if vdense:
            pall = memfirst(jnp.concatenate(p, axis=1))
            uall = jnp.concatenate([urows(h) for h in range(H)], axis=0).astype(BF16)
            for kt in range(H * L // LN):
                t = _dot(pall[:, kt * LN:(kt + 1) * LN], uall[kt * LN:(kt + 1) * LN, :], NN)
                acc = t if acc is None else acc + t
        else:
            for hs in groups:
                npad = LN - L * len(hs)
                pg = memfirst(jnp.concatenate([p[h] for h in hs] + [jnp.zeros((L, npad), F32)], axis=1))
                ug = jnp.concatenate([urows(h) for h in hs] + [jnp.zeros((npad, DM + LN), F32)], axis=0).astype(BF16)
                t = _dot(pg, ug, NN)
                acc = t if acc is None else acc + t
        return acc[M:, :], acc[:M, :]

    def block(b, mem):
        finalize(jnp.maximum(b - 1, 0))
        if unroll == SPB:
            for k in range(SPB):
                a, mem = step(pl.multiple_of(b * TB + k * seg, seg), mem)
                abuf[pl.ds(k * seg, seg), :] = a
        else:
            def inner(k, mem):
                a, mem2 = step(pl.multiple_of(b * TB + k * seg, seg), mem)
                abuf[pl.ds(pl.multiple_of(k * seg, seg), seg), :] = a
                return mem2
            mem = lax.fori_loop(0, SPB, inner, mem, unroll=unroll)
        @pl.when(b > 0)
        def _():
            o_copy(b - 1).start()
        return mem

    with jax.named_scope("steps"):
        lax.fori_loop(0, NB, block, jnp.concatenate([memb[...].astype(F32), jnp.zeros((M, DP - D), F32)], axis=1), unroll=blockunroll)
    with jax.named_scope("epilogue"):
        finalize(NB - 1)
        o_copy(NB - 1).start()
        pltpu.make_async_copy(obuf, obuf, sem_o).wait()

def call(xt, mem0, wq, wk, wv, wot, w1, w2t, *, name, seg=32, unroll=4, nobc=True, dmapos=0, memlast=True, vdense=True, roundmem=True, flags=None, lag=1, mainunroll=0, foldunroll=8, blockunroll=1):
    D, S = xt.shape
    H, _, DH = wot.shape
    M = mem0.shape[0]; Fh = w1.shape[1]
    NB = S // TB
    NC = DH // LN
    DP = (D // LN + 1) * LN
    hbm = pl.BlockSpec(memory_space=pltpu.HBM)
    return pl.pallas_call(
        functools.partial(_kernel, seg=seg, H=H, unroll=unroll, dmapos=dmapos, memlast=memlast, vdense=vdense, roundmem=roundmem, lag=lag, mainunroll=mainunroll, foldunroll=foldunroll, blockunroll=blockunroll),
        out_shape=jax.ShapeDtypeStruct((D, S), BF16),
        in_specs=[hbm] * 8, out_specs=hbm,
        scratch_shapes=[
            pltpu.VMEM((NB, D, TB), BF16), pltpu.VMEM((S, DP), BF16), pltpu.VMEM((NB, D, TB), F32),
            pltpu.VMEM((NB - D // DC, TB, Fh), BF16),
            pltpu.VMEM((3 * NC, D * H, LN), BF16), pltpu.VMEM((H, D, DH), BF16),
            pltpu.VMEM((D, Fh), BF16), pltpu.VMEM((D, Fh), BF16), pltpu.VMEM((M, D), BF16),
            pltpu.VMEM((H * 2 * NC, DP // 2, LN), U32), pltpu.VMEM((H * NC, D // 2, LN), U32),
            pltpu.VMEM(((H // 2) * (2 * (D // LN) + 1), DP // 2, LN), U32),
            pltpu.VMEM((TB, DP), F32), pltpu.VMEM((NB, D, TB), BF16),
            pltpu.SemaphoreType.DMA((NB,)), pltpu.SemaphoreType.DMA((3 * NC, D // (DC * GB))),
            pltpu.SemaphoreType.DMA((4,)), pltpu.SemaphoreType.DMA(()),
        ],
        compiler_params=pltpu.CompilerParams(vmem_limit_bytes=100 * 1024 * 1024, disable_bounds_checks=nobc, flags=flags or {}),
        name=name,
    )(xt, mem0, wq.reshape(D * H, DH), wk.reshape(D * H, DH), wv.reshape(D * H, DH), wot, w1, w2t)


@functools.partial(jax.jit, static_argnames=("A_seg_len",))
def pallas_parallel_sum__memory_aug_recurrent_mem_tr__dense_activation_silu__prompt_kernel(
    A_x: jax.Array,
    A_mem0: jax.Array,
    A_Wq: jax.Array,
    A_Wk: jax.Array,
    A_Wv: jax.Array,
    A_Wo: jax.Array,
    A_seg_len: int,
    B_x: jax.Array,
    B_w1: jax.Array,
    B_w2: jax.Array,
):
    del B_x
    B, S, D = A_x.shape
    M = A_mem0.shape[1]
    assert B == 1 and S % A_seg_len == 0
    x_t = jnp.transpose(A_x, (0, 2, 1)).reshape(D, S)
    wo_t = jnp.transpose(A_Wo, (0, 2, 1))
    out_t = call(x_t, A_mem0.reshape(M, D), A_Wq, A_Wk, A_Wv, wo_t, B_w1, B_w2.T,
                 name="rmt_mlp", seg=A_seg_len)
    return jnp.transpose(out_t.reshape(B, D, S), (0, 2, 1))
```

```python
import functools
import jax
import jax.numpy as jnp
from jax import lax
import jax.experimental.pallas as pl
import jax.experimental.pallas.tpu as pltpu

F32 = jnp.float32
BF16 = jnp.bfloat16
U32 = jnp.uint32
NN = (((1,), (0,)), ((), ()))
NT = (((1,), (1,)), ((), ()))
LOG2E = 1.4426950408889634
TB = 128
GB = 2
DC = 32
FC = 256
LN = 128

def _dot(a, b, dims):
    return lax.dot_general(a, b, dims, preferred_element_type=F32)


def _layernorm_t(xt):
    mu = jnp.mean(xt, axis=0, keepdims=True)
    xc = xt - mu
    var = jnp.mean(xc * xc, axis=0, keepdims=True)
    return xc * lax.rsqrt(var + 1e-5)

def _silu(a):
    h = 0.5 * a
    return h + h * jnp.tanh(h)

def _step_order(n_heads, lag=1, zlag=4, rlag=2):
    big = [("K", i) for i in range(n_heads)] + [("U", p) for p in range(n_heads // 2)]
    out = []
    zdone = []
    for j, b in enumerate(big):
        out.append(b)
        if 0 <= j - lag < n_heads:
            out.append(("S", j - lag))
        for p in range(n_heads // 2):
            if j == 2 * p + 1 + lag + zlag:
                out.append(("Z", p))
            if j == 2 * p + 1 + lag + zlag + rlag:
                out.append(("R", p))
    seen = {o for o in out}
    out += [("Z", p) for p in range(n_heads // 2) if ("Z", p) not in seen]
    out += [("R", p) for p in range(n_heads // 2) if ("R", p) not in seen]
    return out


def _kernel(xt_hbm, mem0_hbm, wq_hbm, wk_hbm, wv_hbm, wot_hbm, w1_hbm, w2t_hbm, ot_hbm,
            xbuf, xnbuf, base, hidb, stage, wob, w1b, w2b, memb, wqk, wvp, wb, wr, abuf, obuf,
            sem_x, sem_w, sem_misc, sem_o, *, seg, H, PRE, CA, lag, foldrem, zlag, rlag):
    D, S = xt_hbm.shape
    DH = wq_hbm.shape[1]
    M = mem0_hbm.shape[0]
    Fh = w1_hbm.shape[1]
    L = M + seg
    NB = S // TB
    SPB = TB // seg
    NJ = D // DC
    NC = DH // LN
    nch = Fh // FC
    DM = (D // LN) * LN
    DR = D - DM
    NM = DM // LN
    DP = DM + LN
    w_hbm = (wq_hbm, wk_hbm, wv_hbm)

    def x_copy(b):
        return pltpu.make_async_copy(xt_hbm.at[:, pl.ds(pl.multiple_of(b * TB, TB), TB)], xbuf.at[b], sem_x.at[b])
    def w_copy(wi, c, j):
        rows = pl.ds(pl.multiple_of(j * (GB * DC * H), GB * DC * H), GB * DC * H)
        return pltpu.make_async_copy(w_hbm[wi].at[rows, pl.ds(c * LN, LN)], stage.at[wi * NC + c, rows], sem_w.at[wi * NC + c, j])
    def o_copy(b):
        return pltpu.make_async_copy(obuf.at[b], ot_hbm.at[:, pl.ds(pl.multiple_of(b * TB, TB), TB)], sem_o)
    FA = CA * FC
    c_w1a = pltpu.make_async_copy(w1_hbm.at[:, pl.ds(0, FA)], w1b.at[:, pl.ds(0, FA)], sem_misc.at[0])
    c_w1b = pltpu.make_async_copy(w1_hbm.at[:, pl.ds(FA, Fh - FA)], w1b.at[:, pl.ds(FA, Fh - FA)], sem_misc.at[4])
    c_w2 = pltpu.make_async_copy(w2t_hbm, w2b, sem_misc.at[1])
    c_wo = pltpu.make_async_copy(wot_hbm, wob, sem_misc.at[2])
    c_mem = pltpu.make_async_copy(mem0_hbm, memb, sem_misc.at[3])
    def w_start(j):
        for wi in range(3):
            for c in range(NC): w_copy(wi, c, j).start()
    def w_wait(j):
        for wi in range(3):
            for c in range(NC): w_copy(wi, c, j).wait()

    NG = NJ // GB
    lax.fori_loop(0, PRE, lambda b, c: (x_copy(b).start(), c)[-1], 0)
    c_w1a.start()
    lax.fori_loop(0, 1, lambda b, c: (c_w1b.start(), x_copy(PRE).start(), c)[-1], 0)
    c_w2.start()
    def first_groups(g, c):
        for k in range(GB):
            x_copy(PRE + 1 + g * GB + k).start()
        w_start(g)
        return c
    lax.fori_loop(0, 2, first_groups, 0)
    lax.fori_loop(PRE + 1 + 2 * GB, NB, lambda b, c: (x_copy(b).start(), c)[-1], 0)

    def ln_block(b):
        xnt = _layernorm_t(xbuf[b].astype(F32))
        xnt = jnp.concatenate([xnt, jnp.zeros((DP - D, TB), F32)], axis=0)
        xnbuf[pl.ds(pl.multiple_of(b * TB, TB), TB), :] = xnt.T.astype(BF16)

    def relayout(j, wi, c, part, dup):
        r16 = pl.multiple_of((j * DC + part * 16) * H, 16 * H)
        src = stage.at[wi * NC + c, pl.ds(r16, 16 * H)].bitcast(U32)
        p0 = pl.multiple_of(j * (DC // 2) + part * 8, 8)
        for hp in range(H // 2):
            even = src[pl.ds(hp, 8, stride=H), :]
            odd = src[pl.ds(hp + H // 2, 8, stride=H), :]
            lo = (even & U32(0xFFFF)) | (odd << 16)
            hi = (even >> 16) | (odd & U32(0xFFFF0000))
            for k, val in enumerate((lo, hi)):
                h = 2 * hp + k
                if wi < 2:
                    wqk[(h * 2 + wi) * NC + c, pl.ds(p0, 8), :] = val
                    if dup:
                        wqk[(h * 2 + wi) * NC + c, pl.ds(p0 + DR // 2, 8), :] = val
                else:
                    wvp[h * NC + c, pl.ds(p0, 8), :] = val

    def up_chunk(xn, c):
        return _silu(_dot(xn, w1b[:, c * FC:(c + 1) * FC], NN)).astype(BF16)

    def load_xn(b):
        return xnbuf[pl.ds(pl.multiple_of(b * TB, TB), TB), :D]

    def mlp_down(b, hid):
        base[b] = xbuf[b].astype(F32) + _dot(w2b[...], hid, NT)

    def mlp_block(b, j, ln_next=True, dup=False):
        xn = load_xn(b)
        if ln_next:
            ln_block(b + 1)
        pieces = [(jj, wi, c, part) for jj in j for wi in range(3) for part in range(DC // 16) for c in range(NC)]
        hid = []
        for c in range(nch):
            hid.append(up_chunk(xn, c))
            for q in range((len(pieces) * c) // nch, (len(pieces) * (c + 1)) // nch):
                relayout(*pieces[q], dup)
        mlp_down(b, jnp.concatenate(hid, axis=1))

    with jax.named_scope("st_x"):
        for b in range(PRE):
            x_copy(b).wait()
    with jax.named_scope("st_ln"):
        for b in range(PRE):
            ln_block(b)
        abuf[...] = jnp.zeros(abuf.shape, F32)
    with jax.named_scope("st_w1a"):
        c_w1a.wait()
    with jax.named_scope("pre_upa"):
        for b in range(PRE):
            xn = load_xn(b)
            hidb[b, :, pl.ds(0, FA)] = jnp.concatenate([up_chunk(xn, c) for c in range(CA)], axis=1)
    with jax.named_scope("st_w1b"):
        c_w1b.wait()
        x_copy(PRE).wait()
    with jax.named_scope("pre_upb"):
        ln_block(PRE)
        for b in range(PRE):
            xn = load_xn(b)
            hidb[b, :, pl.ds(FA, Fh - FA)] = jnp.concatenate([up_chunk(xn, c) for c in range(CA, nch)], axis=1)
    with jax.named_scope("st_w2"):
        c_w2.wait()
    with jax.named_scope("pre_down"):
        for b in range(PRE):
            mlp_down(b, hidb[b])

    def group_body(g, carry):
        w_wait(g)
        @pl.when(g + 2 < NG)
        def _():
            w_start(g + 2)
        @pl.when(g + 2 == NG)
        def _():
            c_wo.start()
            c_mem.start()
        for k in range(GB):
            x_copy(PRE + 1 + g * GB + k).wait()
        lax.fori_loop(g * GB, (g + 1) * GB, lambda j, c: (mlp_block(j + PRE, [j]), c)[-1], 0)
        return carry
    assert (NG - 1) * GB * DC == DM and GB * DC == DR and PRE + (NG - 1) * GB + 1 == NB
    with jax.named_scope("main"):
        lax.fori_loop(0, NG - 1, group_body, 0)
        w_wait(NG - 1)
        mlp_block(NB - 1, list(range((NG - 1) * GB, NJ)), ln_next=False, dup=True)
    with jax.named_scope("waitwo"):
        c_mem.wait(); c_wo.wait()

    def fold_pair(p, carry):
        bs = []
        for k in range(2):
            h = 2 * p + k
            wv_h = jnp.concatenate([pltpu.bitcast(wvp[h * NC + c], BF16) for c in range(NC)], axis=1)
            bs.append(_dot(wv_h, wob[h], NT).astype(BF16))
        tiles = [bs[0][:DM, t * LN:(t + 1) * LN] for t in range(NM)]
        tiles.append(jnp.concatenate([bs[0][:DM, DM:], bs[1][:DM, DM:]], axis=1))
        tiles += [bs[1][:DM, t * LN:(t + 1) * LN] for t in range(NM)]
        for t, tile in enumerate(tiles):
            wb[p * (2 * NM + 1) + t] = pltpu.bitcast(tile, U32)
        both = jnp.concatenate([bs[0][DM:], bs[1][DM:]], axis=0)
        both = jnp.concatenate([both, jnp.zeros((2 * DR, DP - D), BF16)], axis=1)
        for t in range(NM + 1):
            wr[p * (NM + 1) + t] = pltpu.bitcast(both[:, t * LN:(t + 1) * LN], U32)
        return carry
    with jax.named_scope("fold"):
        lax.fori_loop(0, H // 2, fold_pair, 0, unroll=True)

    row = lax.broadcasted_iota(jnp.int32, (L, L), 0)
    col = lax.broadcasted_iota(jnp.int32, (L, L), 1)
    mask = (row >= seg) | (col >= seg) | (row >= col)
    lo_half = lax.broadcasted_iota(jnp.int32, (L, LN), 1) < DR
    scale = DH ** (-0.5)
    order = _step_order(H, lag, zlag, rlag)
    TP = 2 * NM + 1

    def finalize(b):
        a = abuf[...]
        rem = a[:, DM:]
        rem = rem + pltpu.roll(rem, DR, 1)
        at = jnp.concatenate([a[:, :DM].T, rem.T[:DR]], axis=0)
        obuf[b] = (base[b] + at).astype(BF16)

    def step(r0, mem):
        xs = xnbuf[pl.ds(r0, seg), :].astype(F32)
        hcat = jnp.concatenate([xs, mem], axis=0)
        def memfirst(a):
            return jnp.concatenate([a[seg:], a[:seg]], axis=0)
        rem = hcat[:, DM:]
        rem = rem + pltpu.roll(rem, DR, 1)
        zpad = jnp.zeros((DR - L, LN), F32)
        zst = jnp.concatenate([jnp.where(lo_half, rem, 0.0), zpad, jnp.where(lo_half, 0.0, rem), zpad], axis=0).astype(BF16)
        qk = [None] * H; p = [None] * H; u = [None] * (H // 2); z = [None] * (H // 2)
        acc = None
        for kind, i in order:
            if kind == "K":
                w = jnp.concatenate([pltpu.bitcast(wqk[i * 2 * NC + t], BF16) for t in range(2 * NC)], axis=1)
                qk[i] = _dot(hcat, w, NN)
            elif kind == "S":
                sc = _dot(qk[i][:, 0:DH], qk[i][:, DH:2 * DH], NT)
                sc = jnp.where(mask, sc, -1e9 / scale)
                m = jnp.max(sc, axis=-1, keepdims=True)
                e = jnp.exp2((sc - m) * (scale * LOG2E))
                l = jnp.sum(e, axis=-1, keepdims=True)
                r = pl.reciprocal(l, approx=True)
                p[i] = e * (r * (2.0 - l * r))
            elif kind == "U":
                w = jnp.concatenate([pltpu.bitcast(wb[i * TP + t], BF16) for t in range(TP)], axis=1)
                u[i] = _dot(hcat[:, :DM], w, NN)
            elif kind == "Z":
                pz = jnp.zeros((L, DR - L), F32)
                pp = memfirst(jnp.concatenate([p[2 * i], pz, p[2 * i + 1], pz], axis=1))
                z[i] = _dot(pp, zst, NN)
            else:
                w = jnp.concatenate([pltpu.bitcast(wr[i * (NM + 1) + t], BF16) for t in range(NM + 1)], axis=1)
                t = _dot(z[i], w, NN)
                acc = t if acc is None else acc + t
        def urows(h):
            up = u[h // 2]
            rem = up[:, DM:DM + LN]
            if h % 2 == 0:
                return jnp.concatenate([up[:, 0:DM], jnp.where(lo_half, rem, 0.0)], axis=1)
            return jnp.concatenate([up[:, DM + LN:], jnp.where(lo_half, 0.0, rem)], axis=1)
        pall = memfirst(jnp.concatenate(p, axis=1))
        uall = jnp.concatenate([urows(h) for h in range(H)], axis=0).astype(BF16)
        for kt in range(H * L // LN):
            t = _dot(pall[:, kt * LN:(kt + 1) * LN], uall[kt * LN:(kt + 1) * LN, :], NN)
            acc = t if acc is None else acc + t
        return acc[M:, :], acc[:M, :]

    def block(b, mem):
        finalize(jnp.maximum(b - 1, 0))
        for k in range(SPB):
            a, mem = step(pl.multiple_of(b * TB + k * seg, seg), mem)
            abuf[pl.ds(k * seg, seg), :] = a
        @pl.when(b > 0)
        def _():
            o_copy(b - 1).start()
        return mem

    with jax.named_scope("steps"):
        lax.fori_loop(0, NB, block, jnp.concatenate([memb[...].astype(F32), jnp.zeros((M, DP - D), F32)], axis=1))
    with jax.named_scope("epilogue"):
        finalize(NB - 1)
        o_copy(NB - 1).start()
        pltpu.make_async_copy(obuf, obuf, sem_o).wait()

def call(xt, mem0, wq, wk, wv, wot, w1, w2t, *, name, seg=32, PRE=3, CA=3, lag=1, foldrem=False, zlag=4, rlag=2):
    D, S = xt.shape
    H, _, DH = wot.shape
    M = mem0.shape[0]; Fh = w1.shape[1]
    NB = S // TB
    NC = DH // LN
    DP = (D // LN + 1) * LN
    hbm = pl.BlockSpec(memory_space=pltpu.HBM)
    return pl.pallas_call(
        functools.partial(_kernel, seg=seg, H=H, PRE=PRE, CA=CA, lag=lag, foldrem=foldrem, zlag=zlag, rlag=rlag),
        out_shape=jax.ShapeDtypeStruct((D, S), BF16),
        in_specs=[hbm] * 8, out_specs=hbm,
        scratch_shapes=[
            pltpu.VMEM((NB, D, TB), BF16), pltpu.VMEM((S, DP), BF16), pltpu.VMEM((NB, D, TB), F32),
            pltpu.VMEM((PRE, TB, Fh), BF16),
            pltpu.VMEM((3 * NC, D * H, LN), BF16), pltpu.VMEM((H, D, DH), BF16),
            pltpu.VMEM((D, Fh), BF16), pltpu.VMEM((D, Fh), BF16), pltpu.VMEM((M, D), BF16),
            pltpu.VMEM((H * 2 * NC, DP // 2, LN), U32), pltpu.VMEM((H * NC, D // 2, LN), U32),
            pltpu.VMEM(((H // 2) * (2 * (D // LN) + 1), (D // LN) * LN // 2, LN), U32),
            pltpu.VMEM(((H // 2) * (D // LN + 1), LN // 2, LN), U32),
            pltpu.VMEM((TB, DP), F32), pltpu.VMEM((NB, D, TB), BF16),
            pltpu.SemaphoreType.DMA((NB,)), pltpu.SemaphoreType.DMA((3 * NC, D // (DC * GB))),
            pltpu.SemaphoreType.DMA((5,)), pltpu.SemaphoreType.DMA(()),
        ],
        compiler_params=pltpu.CompilerParams(vmem_limit_bytes=100 * 1024 * 1024, disable_bounds_checks=True),
        name=name,
    )(xt, mem0, wq.reshape(D * H, DH), wk.reshape(D * H, DH), wv.reshape(D * H, DH), wot, w1, w2t)


@functools.partial(jax.jit, static_argnames=("A_seg_len",))
def pallas_parallel_sum__memory_aug_recurrent_mem_tr__dense_activation_silu__prompt_kernel(
    A_x: jax.Array,
    A_mem0: jax.Array,
    A_Wq: jax.Array,
    A_Wk: jax.Array,
    A_Wv: jax.Array,
    A_Wo: jax.Array,
    A_seg_len: int,
    B_x: jax.Array,
    B_w1: jax.Array,
    B_w2: jax.Array,
):
    del B_x
    B, S, D = A_x.shape
    M = A_mem0.shape[1]
    assert B == 1 and S % A_seg_len == 0
    x_t = jnp.transpose(A_x, (0, 2, 1)).reshape(D, S)
    wo_t = jnp.transpose(A_Wo, (0, 2, 1))
    out_t = call(x_t, A_mem0.reshape(M, D), A_Wq, A_Wk, A_Wv, wo_t, B_w1, B_w2.T,
                 name="rmt_mlp", seg=A_seg_len)
    return jnp.transpose(out_t.reshape(B, D, S), (0, 2, 1))
```

```python
import functools

import jax
import jax.numpy as jnp
import numpy as np
from jax import lax
import jax.experimental.pallas as pl
import jax.experimental.pallas.tpu as pltpu

F32 = jnp.float32
BF16 = jnp.bfloat16
U32 = jnp.uint32
NN = (((1,), (0,)), ((), ()))
NT = (((1,), (1,)), ((), ()))
LOG2E = 1.4426950408889634
LO16 = np.uint32(0x0000FFFF)
HI16 = np.uint32(0xFFFF0000)

LANES = 128
TB = 128
FC = 256
CA = 3
PRE = 3
DC = 32
GB = 2


def _dot(a, b, dims):
    return lax.dot_general(a, b, dims, preferred_element_type=F32)


def _layernorm_t(xt):
    mu = jnp.mean(xt, axis=0, keepdims=True)
    xc = xt - mu
    var = jnp.mean(xc * xc, axis=0, keepdims=True)
    return xc * lax.rsqrt(var + 1e-5)


def _silu(a):
    h = 0.5 * a
    return h + h * jnp.tanh(h)


def _step_order(n_heads, lag=1, zlag=4, rlag=2):
    big = [("K", h) for h in range(n_heads)] + [("U", p) for p in range(n_heads // 2)]
    out = []
    for j, b in enumerate(big):
        out.append(b)
        if 0 <= j - lag < n_heads:
            out.append(("S", j - lag))
        for p in range(n_heads // 2):
            if j == 2 * p + 1 + lag + zlag:
                out.append(("Z", p))
            if j == 2 * p + 1 + lag + zlag + rlag:
                out.append(("R", p))
    out += [("Z", p) for p in range(n_heads // 2) if ("Z", p) not in out]
    out += [("R", p) for p in range(n_heads // 2) if ("R", p) not in out]
    return out


def _kernel(xt_hbm, mem0_hbm, wq_hbm, wk_hbm, wv_hbm, wot_hbm, w1_hbm, w2t_hbm, ot_hbm,
            xbuf, xnbuf, base, hidb, stage, wob, w1a, w1b, w2b, memb, wqk, wvp, wb, wr, abuf, obuf,
            sem_x, sem_w, sem_misc, sem_o, *, seg):
    D, S = xt_hbm.shape
    H = wot_hbm.shape[0]
    DH = wq_hbm.shape[1]
    M = mem0_hbm.shape[0]
    Fh = w1_hbm.shape[1]
    L = M + seg
    NB = S // TB
    SPB = TB // seg
    NG = D // (DC * GB)
    NC = DH // LANES
    nch = Fh // FC
    FA = CA * FC
    NM = D // LANES
    DM = NM * LANES
    DR = D - DM
    DP = DM + LANES
    TP = 2 * NM + 1
    w_hbm = (wq_hbm, wk_hbm, wv_hbm)

    def x_copy(b):
        cols = pl.ds(pl.multiple_of(b * TB, TB), TB)
        return pltpu.make_async_copy(xt_hbm.at[:, cols], xbuf.at[b], sem_x.at[b])

    def o_copy(b):
        cols = pl.ds(pl.multiple_of(b * TB, TB), TB)
        return pltpu.make_async_copy(obuf.at[b], ot_hbm.at[:, cols], sem_o)

    def w_copies(g):
        rows = pl.ds(pl.multiple_of(g * (GB * DC * H), GB * DC * H), GB * DC * H)
        return [pltpu.make_async_copy(w_hbm[wi].at[rows, pl.ds(c * LANES, LANES)],
                                      stage.at[wi * NC + c, rows], sem_w.at[wi * NC + c, g])
                for wi in range(3) for c in range(NC)]

    def w_start(g):
        for cp in w_copies(g):
            cp.start()

    def w_wait(g):
        for cp in w_copies(g):
            cp.wait()

    c_w1a = pltpu.make_async_copy(w1_hbm.at[:, pl.ds(0, FA)], w1a, sem_misc.at[0])
    c_w1b = pltpu.make_async_copy(w1_hbm.at[:, pl.ds(FA, Fh - FA)], w1b, sem_misc.at[1])
    c_w2 = pltpu.make_async_copy(w2t_hbm, w2b, sem_misc.at[2])
    c_wo = pltpu.make_async_copy(wot_hbm, wob, sem_misc.at[3])
    c_mem = pltpu.make_async_copy(mem0_hbm, memb, sem_misc.at[4])

    def x_start_range(lo, hi):
        def body(b, carry):
            x_copy(b).start()
            return carry
        lax.fori_loop(lo, hi, body, 0)

    def first_groups(g, carry):
        for k in range(GB):
            x_copy(PRE + GB + g * GB + k).start()
        w_start(g)
        return carry

    x_start_range(0, PRE)
    c_w1a.start()
    c_w1b.start()
    x_start_range(PRE, PRE + GB)
    c_w2.start()
    lax.fori_loop(0, 2, first_groups, 0)
    x_start_range(PRE + 3 * GB, NB)

    def ln_block(b):
        xnt = _layernorm_t(xbuf[b].astype(F32))
        xnt = jnp.concatenate([xnt, jnp.zeros((DP - D, TB), F32)], axis=0)
        xnbuf[pl.ds(pl.multiple_of(b * TB, TB), TB), :] = xnt.T.astype(BF16)

    def relayout(j, wi, c, part, dup):
        r16 = pl.multiple_of((j * DC + part * 16) * H, 16 * H)
        src = stage.at[wi * NC + c, pl.ds(r16, 16 * H)].bitcast(U32)
        p0 = pl.multiple_of(j * (DC // 2) + part * 8, 8)
        for hp in range(H // 2):
            even = src[pl.ds(hp, 8, stride=H), :]
            odd = src[pl.ds(hp + H // 2, 8, stride=H), :]
            lo = (even & LO16) | (odd << 16)
            hi = (even >> 16) | (odd & HI16)
            for k, val in enumerate((lo, hi)):
                h = 2 * hp + k
                if wi < 2:
                    wqk[(h * 2 + wi) * NC + c, pl.ds(p0, 8), :] = val
                    if dup:
                        wqk[(h * 2 + wi) * NC + c, pl.ds(p0 + DR // 2, 8), :] = val
                else:
                    wvp[h * NC + c, pl.ds(p0, 8), :] = val

    def up_chunk(xn, c):
        w = w1a[:, c * FC:(c + 1) * FC] if c < CA else w1b[:, (c - CA) * FC:(c - CA + 1) * FC]
        return _silu(_dot(xn, w, NN)).astype(BF16)

    def load_xn(b, nblk=1):
        return xnbuf[pl.ds(pl.multiple_of(b * TB, TB), nblk * TB), :D]

    def mlp_blocks(b, nblk, batches, ln_next, dup):
        xn = load_xn(b, nblk)
        if ln_next:
            for k in range(nblk):
                ln_block(jnp.minimum(b + nblk + k, NB - 1))
        pieces = [(j, wi, c, part) for j in batches for wi in range(3)
                  for part in range(DC // 16) for c in range(NC)]
        hid = []
        for c in range(nch):
            hid.append(up_chunk(xn, c))
            for q in range((len(pieces) * c) // nch, (len(pieces) * (c + 1)) // nch):
                relayout(*pieces[q], dup)
        y = _dot(w2b[...], jnp.concatenate(hid, axis=1), NT)
        for k in range(nblk):
            base[b + k] = xbuf[b + k].astype(F32) + y[:, k * TB:(k + 1) * TB]

    for b in range(PRE):
        x_copy(b).wait()
    for b in range(PRE):
        ln_block(b)
    abuf[...] = jnp.zeros(abuf.shape, F32)
    c_w1a.wait()
    for b in range(PRE):
        xn = load_xn(b)
        hidb[b, :, pl.ds(0, FA)] = jnp.concatenate([up_chunk(xn, c) for c in range(CA)], axis=1)
    c_w1b.wait()
    for b in range(PRE, PRE + GB):
        x_copy(b).wait()
    for b in range(PRE, PRE + GB):
        ln_block(b)
    for b in range(PRE):
        xn = load_xn(b)
        hidb[b, :, pl.ds(FA, Fh - FA)] = jnp.concatenate([up_chunk(xn, c) for c in range(CA, nch)], axis=1)
    c_w2.wait()
    for b in range(PRE):
        base[b] = xbuf[b].astype(F32) + _dot(w2b[...], hidb[b], NT)

    def group_body(g, carry):
        w_wait(g)

        @pl.when(g + 2 < NG)
        def _():
            w_start(g + 2)

        @pl.when(g + 2 == NG)
        def _():
            c_wo.start()
            c_mem.start()

        for k in range(GB):
            b = PRE + GB + g * GB + k

            @pl.when(b < NB)
            def _():
                x_copy(jnp.minimum(b, NB - 1)).wait()

        def body(gg, c):
            mlp_blocks(PRE + gg * GB, GB, [gg * GB + k for k in range(GB)], True, False)
            return c
        lax.fori_loop(g, g + 1, body, 0)
        return carry

    assert (NG - 1) * GB * DC == DM and GB * DC == DR and PRE + (NG - 1) * GB + 1 == NB
    lax.fori_loop(0, NG - 1, group_body, 0)
    w_wait(NG - 1)
    mlp_blocks(NB - 1, 1, list(range((NG - 1) * GB, NG * GB)), False, True)
    c_mem.wait()
    c_wo.wait()

    for p in range(H // 2):
        wv = [jnp.concatenate([pltpu.bitcast(wvp[(2 * p + k) * NC + c], BF16) for c in range(NC)], axis=1)
              for k in range(2)]
        bt = [_dot(wob[2 * p + k, DM:], wv[k], NT) for k in range(2)]
        bm = [_dot(wv[k], wob[2 * p + k, :DM], NT).astype(BF16) for k in range(2)]
        rem = jnp.concatenate(bt, axis=0).T
        tiles = [bm[0][:DM, t * LANES:(t + 1) * LANES] for t in range(NM)]
        tiles.append(rem[:DM].astype(BF16))
        tiles += [bm[1][:DM, t * LANES:(t + 1) * LANES] for t in range(NM)]
        for t, tile in enumerate(tiles):
            wb[p * TP + t] = pltpu.bitcast(tile, U32)
        for t in range(NM):
            both = jnp.concatenate([bm[0][DM:, t * LANES:(t + 1) * LANES],
                                    bm[1][DM:, t * LANES:(t + 1) * LANES]], axis=0)
            wr[p * (NM + 1) + t] = pltpu.bitcast(both, U32)
        rr = rem[DM:]
        low = lax.broadcasted_iota(jnp.int32, (DR, LANES), 1) < DR
        both = jnp.concatenate([jnp.where(low, rr, 0.0),
                                jnp.where(low, pltpu.roll(rr, DR, 1), 0.0)], axis=0)
        wr[p * (NM + 1) + NM] = pltpu.bitcast(both.astype(BF16), U32)

    row = lax.broadcasted_iota(jnp.int32, (L, L), 0)
    col = lax.broadcasted_iota(jnp.int32, (L, L), 1)
    mask = (row >= seg) | (col >= seg) | (row >= col)
    lo_half = lax.broadcasted_iota(jnp.int32, (L, LANES), 1) < DR
    scale = DH ** (-0.5)
    order = _step_order(H)

    def packed(ref, first, n):
        return jnp.concatenate([pltpu.bitcast(ref[first + t], BF16) for t in range(n)], axis=1)

    def mem_first(a):
        return jnp.concatenate([a[seg:], a[:seg]], axis=0)

    def step(r0, mem):
        xs = xnbuf[pl.ds(r0, seg), :].astype(F32)
        hcat = jnp.concatenate([xs, mem], axis=0)
        rem = hcat[:, DM:]
        rem = rem + pltpu.roll(rem, DR, 1)
        zpad = jnp.zeros((DR - L, LANES), F32)
        zst = jnp.concatenate([jnp.where(lo_half, rem, 0.0), zpad,
                               jnp.where(lo_half, 0.0, rem), zpad], axis=0).astype(BF16)
        qk = [None] * H
        p = [None] * H
        u = [None] * (H // 2)
        z = [None] * (H // 2)
        acc = None
        for kind, i in order:
            if kind == "K":
                qk[i] = _dot(hcat, packed(wqk, i * 2 * NC, 2 * NC), NN)
            elif kind == "S":
                sc = _dot(qk[i][:, 0:DH], qk[i][:, DH:2 * DH], NT)
                sc = jnp.where(mask, sc, -1e9 / scale)
                m = jnp.max(sc, axis=-1, keepdims=True)
                e = jnp.exp2((sc - m) * (scale * LOG2E))
                l = jnp.sum(e, axis=-1, keepdims=True)
                p[i] = e * (1.0 / l)
            elif kind == "U":
                u[i] = _dot(hcat[:, :DM], packed(wb, i * TP, TP), NN)
            elif kind == "Z":
                pz = jnp.zeros((L, DR - L), F32)
                pp = mem_first(jnp.concatenate([p[2 * i], pz, p[2 * i + 1], pz], axis=1))
                z[i] = _dot(pp, zst, NN)
            else:
                t = _dot(z[i], packed(wr, i * (NM + 1), NM + 1), NN)
                acc = t if acc is None else acc + t

        def u_rows(h):
            up = u[h // 2]
            tail = up[:, DM:DM + LANES]
            if h % 2 == 0:
                return jnp.concatenate([up[:, 0:DM], jnp.where(lo_half, tail, 0.0)], axis=1)
            return jnp.concatenate([up[:, DM + LANES:], jnp.where(lo_half, 0.0, tail)], axis=1)

        pall = mem_first(jnp.concatenate(p, axis=1))
        uall = jnp.concatenate([u_rows(h) for h in range(H)], axis=0).astype(BF16)
        for kt in range(H * L // LANES):
            t = _dot(pall[:, kt * LANES:(kt + 1) * LANES], uall[kt * LANES:(kt + 1) * LANES, :], NN)
            acc = t if acc is None else acc + t
        return acc[M:, :], acc[:M, :]

    def finalize(b):
        a = abuf[...]
        rem = a[:, DM:]
        rem = rem + pltpu.roll(rem, DR, 1)
        at = jnp.concatenate([a[:, :DM].T, rem.T[:DR]], axis=0)
        obuf[b] = (base[b] + at).astype(BF16)

    def block(b, mem):
        finalize(jnp.maximum(b - 1, 0))
        for k in range(SPB):
            a, mem = step(pl.multiple_of(b * TB + k * seg, seg), mem)
            abuf[pl.ds(k * seg, seg), :] = a

        @pl.when(b > 0)
        def _():
            o_copy(b - 1).start()

        return mem

    mem0 = jnp.concatenate([memb[...].astype(F32), jnp.zeros((M, DP - D), F32)], axis=1)
    lax.fori_loop(0, NB, block, mem0)
    finalize(NB - 1)
    o_copy(NB - 1).start()
    pltpu.make_async_copy(obuf, obuf, sem_o).wait()


@functools.partial(jax.jit, static_argnames=("A_seg_len",))
def pallas_parallel_sum__memory_aug_recurrent_mem_tr__dense_activation_silu__prompt_kernel(
    A_x: jax.Array,
    A_mem0: jax.Array,
    A_Wq: jax.Array,
    A_Wk: jax.Array,
    A_Wv: jax.Array,
    A_Wo: jax.Array,
    A_seg_len: int,
    B_x: jax.Array,
    B_w1: jax.Array,
    B_w2: jax.Array,
):
    del B_x
    B, S, D = A_x.shape
    _, H, DH = A_Wq.shape
    M = A_mem0.shape[1]
    Fh = B_w1.shape[1]
    NB = S // TB
    NC = DH // LANES
    NM = D // LANES
    DP = (NM + 1) * LANES
    assert B == 1 and TB % A_seg_len == 0
    hbm = pl.BlockSpec(memory_space=pltpu.HBM)
    out_t = pl.pallas_call(
        functools.partial(_kernel, seg=A_seg_len),
        out_shape=jax.ShapeDtypeStruct((D, S), BF16),
        in_specs=[hbm] * 8,
        out_specs=hbm,
        scratch_shapes=[
            pltpu.VMEM((NB, D, TB), BF16),
            pltpu.VMEM((S, DP), BF16),
            pltpu.VMEM((NB, D, TB), F32),
            pltpu.VMEM((PRE, TB, Fh), BF16),
            pltpu.VMEM((3 * NC, D * H, LANES), BF16),
            pltpu.VMEM((H, D, DH), BF16),
            pltpu.VMEM((D, CA * FC), BF16),
            pltpu.VMEM((D, Fh - CA * FC), BF16),
            pltpu.VMEM((D, Fh), BF16),
            pltpu.VMEM((M, D), BF16),
            pltpu.VMEM((H * 2 * NC, DP // 2, LANES), U32),
            pltpu.VMEM((H * NC, D // 2, LANES), U32),
            pltpu.VMEM(((H // 2) * (2 * NM + 1), NM * LANES // 2, LANES), U32),
            pltpu.VMEM(((H // 2) * (NM + 1), LANES // 2, LANES), U32),
            pltpu.VMEM((TB, DP), F32),
            pltpu.VMEM((NB, D, TB), BF16),
            pltpu.SemaphoreType.DMA((NB,)),
            pltpu.SemaphoreType.DMA((3 * NC, D // (DC * GB))),
            pltpu.SemaphoreType.DMA((5,)),
            pltpu.SemaphoreType.DMA(()),
        ],
        compiler_params=pltpu.CompilerParams(vmem_limit_bytes=100 * 1024 * 1024, disable_bounds_checks=True),
        name="rmt_mlp",
    )(jnp.transpose(A_x, (0, 2, 1)).reshape(D, S), A_mem0.reshape(M, D),
      A_Wq.reshape(D * H, DH), A_Wk.reshape(D * H, DH), A_Wv.reshape(D * H, DH),
      jnp.transpose(A_Wo, (0, 2, 1)), B_w1, B_w2.T)
    return jnp.transpose(out_t.reshape(B, D, S), (0, 2, 1))
```
